```python
import os as _os
_os.environ.setdefault("JAX_PLATFORMS", "cpu")
import jax
import jax.numpy as jnp

def _softmax(x, axis=-1):
    return jax.nn.softmax(x, axis=axis)
def _gelu(x):
    return jax.nn.gelu(x, approximate=True)
def _silu(x):
    return jax.nn.silu(x)
def _sigmoid(x):
    return jax.nn.sigmoid(x)
def _layernorm(x, axis=-1, eps=1e-5):
    m = jnp.mean(x, axis=axis, keepdims=True)
    v = jnp.var(x, axis=axis, keepdims=True)
    return (x - m) / jnp.sqrt(v + eps)
def _scatter_add(tgt, idx, src, axis=0):
    return tgt.at[idx].add(src)
def _segment_sum(src, seg, n):
    return jax.ops.segment_sum(src, seg, n)
class _Rng:
    def __init__(self, key):
        self._k = key
    def _next(self):
        self._k, sub = jax.random.split(self._k)
        return sub
    def normal(self, shape):
        return jax.random.normal(self._next(), shape, dtype=jnp.bfloat16)
    def randint(self, lo, hi, shape):
        return jax.random.randint(self._next(), shape, lo, hi, dtype=jnp.int32)
    def uniform(self, shape, lo=0.0, hi=1.0):
        return jax.random.uniform(self._next(), shape, jnp.bfloat16, lo, hi)
    def permutation(self, n):
        return jax.random.permutation(self._next(), n)


kernel_name = 'parallel_sum__sliding_local_dilated__geglu_ffn__prompt'

def setup_inputs():
    _rng = _Rng(jax.random.key(int.from_bytes(__import__("os").urandom(4), "little")))
    _w = (lambda a: (lambda t: t.astype(jnp.bfloat16) if jnp.issubdtype(t.dtype, jnp.floating) else t)(jnp.asarray(a)))
    def _A_setup():
        B, S, D = 1, 2048, 640
        return {
            "x": _w((lambda *s: _rng.normal(s) * 0.05)(B, S, D)),
            "wqkv": _w((lambda *s: _rng.normal(s) * 0.05)(D, 3 * D)),
            "wo": _w((lambda *s: _rng.normal(s) * 0.05)(D, D)),
        }
    _A_in = _A_setup()

    def _B_setup():
        B, S, D, F = 1, 2048, 640, 1728
        return {
            "x": _w((lambda *s: _rng.normal(s) * 0.05)(B, S, D)),
            "w_gate": _w((lambda *s: _rng.normal(s) * 0.05)(D, F)),
            "w_up": _w((lambda *s: _rng.normal(s) * 0.05)(D, F)),
            "w_down": _w((lambda *s: _rng.normal(s) * 0.05)(F, D)),
        }
    _B_in = _B_setup()

    return {
        "A_x": _A_in["x"],
        "A_wqkv": _A_in["wqkv"],
        "A_wo": _A_in["wo"],
        "B_x": _B_in["x"],
        "B_w_gate": _B_in["w_gate"],
        "B_w_up": _B_in["w_up"],
        "B_w_down": _B_in["w_down"],
    }

def reference(A_x, A_wqkv, A_wo, B_x, B_w_gate, B_w_up, B_w_down):
    def _A_ref(x, wqkv, wo):
        B, S, D = x.shape
        H = 32; Dh = D // H
        W, dil = 8, 2
        qkv = (lambda x, *d: x.transpose(*d))((x @ wqkv).reshape(B, S, 3, H, Dh), 2, 0, 3, 1, 4)
        q, k, v = qkv[0], qkv[1], qkv[2]
        scale = Dh ** -0.5
        pos = jnp.arange(S)
        off = jnp.arange(W) * dil
        idx = pos[:, None] - off[None, :]
        mask = idx >= 0
        idx_c = jnp.where(mask, idx, 0).reshape(-1)
        kg = k[:, :, idx_c, :].reshape(B, H, S, W, Dh)
        vg = v[:, :, idx_c, :].reshape(B, H, S, W, Dh)
        logits = jnp.einsum("bhsd,bhswd->bhsw", q, kg) * scale
        logits = jnp.where(mask[None, None, :, :], logits, -1e9)
        attn = _softmax(logits, axis=-1)
        o = jnp.einsum("bhsw,bhswd->bhsd", attn, vg)
        return (lambda x, *d: x.transpose(*d))(o, 0, 2, 1, 3).reshape(B, S, D) @ wo

    def _B_ref(x, w_gate, w_up, w_down):
        return (_gelu(x @ w_gate) * (x @ w_up)) @ w_down

    x = A_x
    xn = _layernorm(x, axis=-1)
    return x + _A_ref(xn, A_wqkv, A_wo) + _B_ref(xn, B_w_gate, B_w_up, B_w_down)
```

```python
import functools
import math
import jax
import jax.numpy as jnp
from jax import lax
import jax.experimental.pallas as pl
import jax.experimental.pallas.tpu as pltpu

S, D, F, H, DH, W, DIL = 2048, 640, 1728, 32, 20, 8, 2
NT = D // 128
TM0 = 512
TM1 = 384
NB1 = (S - TM0) // TM1
assert TM0 + NB1 * TM1 == S and TM1 <= TM0
HALO = 16
FM = 1664
FT = F - FM
LOG2E = math.log2(math.e)
QSCALE = DH ** -0.5 * LOG2E
NEG = -1e9 * LOG2E
F32 = jnp.float32
BF16 = jnp.bfloat16
U32 = jnp.uint32
GELU_C1 = math.sqrt(2.0 / math.pi)
GELU_C2 = GELU_C1 * 0.044715
RA = 8
SWQ = 2
SWV = 2
PIPE = 1
SPAN = 130
T0 = 0
SPAN0 = 125
ONLY0 = 0
OUTSPLIT = 1

CHUNKS = [(0, 128)] + [(128 + 256 * i, 256) for i in range(6)] + [(FM, FT)]
NCH = len(CHUNKS)
TAIL = NCH - 1
STG = S // 2
FEN = STG + TM1 // 2


def dot_nn(a, b):
    return jnp.dot(a, b, preferred_element_type=F32)


def dot_nt(a, b):
    return lax.dot_general(a, b, (((1,), (1,)), ((), ())), preferred_element_type=F32)


def geglu2(g, u):
    inner = g * (GELU_C1 + GELU_C2 * (g * g))
    a = g * u
    return a + a * jnp.tanh(inner)


def b16(v):
    return pltpu.bitcast(v, BF16)


def u32(v):
    return pltpu.bitcast(v, U32)


def kernel(x_hbm, wqkv_hbm, wo_hbm, wgt_hbm, wut_hbm, wd_hbm, out_hbm,
           xx, xn_scr, wqkv_v, wo_v, wgu_v, wd_v, wqkvp, wop, t_scr, a_scr, out_v, z_smem,
           sem_i, sem_o):
    z_smem[0] = 0
    nsem = [0]
    x_u, wqkv_u, wo_u, wgt_u, wut_u, wd_u, out_u = [
        r.bitcast(U32) for r in (x_hbm, wqkv_hbm, wo_hbm, wgt_hbm, wut_hbm, wd_hbm, out_hbm)]

    def in_copy(src, dst):
        c = pltpu.make_async_copy(src, dst, sem_i.at[nsem[0]])
        nsem[0] += 1
        return c

    def out_copy(b, prow, j):
        if OUTSPLIT:
            cols = pl.ds(j * 128, 128)
            return pltpu.make_async_copy(out_v.at[prow, cols], out_u.at[prow, cols], sem_o.at[b * NT + j])
        return pltpu.make_async_copy(out_v.at[prow], out_u.at[prow], sem_o.at[b * NT])

    def x_copy(lo, hi):
        return [in_copy(x_u.at[pl.ds(lo // 2, (hi - lo) // 2)], xx.at[pl.ds(lo // 2, (hi - lo) // 2)])]

    def gu_copy(ci):
        c0, cs = CHUNKS[ci]
        return [in_copy(wgt_u.at[pl.ds(c0 // 2, cs // 2)], wgu_v.at[pl.ds(c0, cs // 2)]),
                in_copy(wut_u.at[pl.ds(c0 // 2, cs // 2)], wgu_v.at[pl.ds(c0 + cs // 2, cs // 2)])]

    def wqkv_copy(lo, hi):
        return [in_copy(wqkv_u.at[:, pl.ds(lo * D, (hi - lo) * D)], wqkv_v.at[:, pl.ds(lo * D, (hi - lo) * D)])]

    groups = [
        x_copy(0, TM0 // 2),
        x_copy(TM0 // 2, TM0),
        gu_copy(0),
        gu_copy(1),
        gu_copy(2) + wqkv_copy(0, 1),
        gu_copy(3) + gu_copy(TAIL) + wqkv_copy(1, 3),
        gu_copy(4) + gu_copy(5) + gu_copy(6) + x_copy(TM0, TM0 + TM1) + [in_copy(wo_u, wo_v)],
        [in_copy(wd_u, wd_v)] + x_copy(TM0 + TM1, S),
    ]

    def wait(g):
        for c in groups[g]:
            c.wait()

    def ln_rows(src, n):
        x = b16(xx[pl.ds(src, n // 2), :]).astype(F32)
        m = jnp.sum(x, axis=-1, keepdims=True) * (1.0 / D)
        xc = x - m
        var = jnp.sum(xc * xc, axis=-1, keepdims=True) * (1.0 / D)
        return xc * lax.rsqrt(var + 1e-5)

    def ln_x(src):
        return b16(xx[pl.ds(src, 8), :]).astype(F32)

    def ln_s1(src):
        return jnp.broadcast_to(jnp.sum(ln_x(src), axis=-1, keepdims=True) * (1.0 / D), (16, 128))

    def ln_s2(src, m):
        xc = ln_x(src) - jnp.concatenate([m] * NT, axis=1)
        var = jnp.sum(xc * xc, axis=-1, keepdims=True) * (1.0 / D)
        return jnp.broadcast_to(lax.rsqrt(var + 1e-5), (16, 128))

    def ln_s3(src, dst, m, rs):
        y = (ln_x(src) - jnp.concatenate([m] * NT, axis=1)) * jnp.concatenate([rs] * NT, axis=1)
        xx[pl.ds(dst, 8), :] = u32(y.astype(BF16))
        return y[:, 0:128]

    def fence_x(val8, z):
        xx[pl.ds(pl.multiple_of(FEN + z, 8), 8), 0:128] = u32(val8)

    def fence_a(val8, z):
        a_scr[3 * NT, pl.ds(pl.multiple_of(z, 8), 8), :] = val8

    def publish_xn():
        xn_scr[0:TM1 // 2, :] = xx[STG:STG + TM1 // 2, :]

    def get_xn(tm):
        return b16(xn_scr[0:tm // 2, :])

    def prep_qkv(p):
        for c in range(NT):
            bt = b16(wqkv_v[:, p * D + c * 128: p * D + (c + 1) * 128]).astype(F32).T
            for j in range(NT):
                t_scr[p, j, c * 128:(c + 1) * 128, :] = bt[:, j * 128:(j + 1) * 128]
        for d in range(DH):
            for j in range(NT):
                rows = t_scr[p, j, pl.ds(d, H, stride=DH), :]
                wqkvp[(p * D + d * H) // 2: (p * D + (d + 1) * H) // 2, j * 128:(j + 1) * 128] = u32(rows.astype(BF16))

    def prep_wo():
        for j in range(NT):
            t_scr[0, j] = b16(wo_v[:, j * 128:(j + 1) * 128]).astype(F32)
        for d in range(DH):
            for j in range(NT):
                rows = t_scr[0, j, pl.ds(d, H, stride=DH), :]
                wop[d * H // 2:(d + 1) * H // 2, j * 128:(j + 1) * 128] = u32(rows.astype(BF16))

    def proj(tm, p, j0=0, j1=NT):
        y = dot_nt(get_xn(tm), b16(wqkvp[(p * D + j0 * 128) // 2:(p * D + j1 * 128) // 2, :]))
        if p == 0:
            y = y * QSCALE
        for j in range(j0, j1):
            a_scr[p * NT + j, HALO:HALO + tm, :] = y[:, (j - j0) * 128:(j - j0 + 1) * 128]

    def att_qk(first, r, z):
        q = a_scr[0:NT, HALO + r:HALO + r + RA, :]
        s = []
        for w in range(W):
            lo = HALO + r - DIL * w
            sw = jnp.sum(q * a_scr[NT:2 * NT, lo:lo + RA, :], axis=0)
            if (w + 1) % SWQ == 0:
                fence_a(sw, z)
            t = sw + pltpu.roll(sw, 64, 1)
            s.append(t + pltpu.roll(t, 32, 1))
        if first and r < DIL * (W - 1):
            pos = r + lax.broadcasted_iota(jnp.int32, (RA, 128), 0)
            s = [jnp.where(pos >= DIL * w, s[w], NEG) for w in range(W)]
        return s

    def att_pv(r, z, s):
        mx = functools.reduce(jnp.maximum, s)
        p = [jnp.exp2(l - mx) for l in s]
        den = functools.reduce(lambda a, b: a + b, p)
        inv = pl.reciprocal(den, approx=True)
        inv = inv * (2.0 - den * inv)
        o = None
        for w in range(W):
            lo = HALO + r - DIL * w
            t = p[w][None] * a_scr[2 * NT:3 * NT, lo:lo + RA, :]
            o = t if o is None else o + t
            if (w + 1) % SWV == 0 and w < W - 1:
                fence_a(o[NT - 1], z)
        a_scr[0:NT, pl.ds(pl.multiple_of(HALO + r + z, 8), RA), :] = o * inv[None]

    class Att:
        def __init__(self, tm, first, z, passes, t0, span, nsrc):
            self.tm, self.first, self.z, self.passes, self.t0, self.span = tm, first, z, passes, t0, span
            self.rows = list(range(0, tm, RA))
            self.n = len(self.rows) + PIPE
            self.i = 0
            self.pend = []
            self.nsrc = nsrc
            self.m = self.rs = None
            self.link = []

        def step(self, trig=None):
            i, z = self.i, self.z
            c = i // 2
            nln = TM1 // 16
            if trig is not None:
                fence_a(trig, z)
                if c <= nln:
                    fence_x(trig, z)
            for v in self.link:
                fence_a(v[0:8], z)
                fence_a(v[8:16], z)
            self.link = []
            if i % 2 == 0:
                if 0 < c <= nln:
                    self.link.append(ln_s3(self.nsrc + (c - 1) * 8, STG + (c - 1) * 8, self.m, self.rs))
                if c < nln:
                    self.m = ln_s1(self.nsrc + c * 8)
                    self.link.append(self.m)
            elif c < nln:
                self.rs = ln_s2(self.nsrc + c * 8, self.m)
                self.link.append(self.rs)
            if i < len(self.rows):
                self.pend.append((self.rows[i], att_qk(self.first, self.rows[i], z)))
            if i >= PIPE:
                r0, s0 = self.pend.pop(0)
                att_pv(r0, z, s0)
            self.i = i + 1

        def emit(self, res, npass):
            for j in range(res.shape[1] // 128):
                rnd = (self.passes + npass - 1) // 4
                self.passes += npass
                while self.i < self.n and self.t0 + self.span * self.i / self.n < 4 * (rnd + 1):
                    frac = max(0.0, (self.t0 + self.span * self.i / self.n - 4 * rnd) / 4)
                    tr = min(self.tm - 8, int(frac * self.tm) // 8 * 8)
                    self.step(res[tr:tr + 8, j * 128:(j + 1) * 128] if self.i > 0 else None)

        def flush(self):
            while self.i < self.n:
                self.step()
            a_scr[NT:3 * NT, 0:HALO, :] = a_scr[NT:3 * NT, self.tm:self.tm + HALO, :]

    def gu_chunk(tm, ci, z=None):
        c0, cs = CHUNKS[ci]
        if z is not None:
            gu = jnp.concatenate([
                dot_nt(b16(xn_scr[0:tm // 4, :]), b16(wgu_v[c0:c0 + cs, :])),
                dot_nt(b16(xn_scr[tm // 4:tm // 2, :]), b16(wgu_v[pl.ds(pl.multiple_of(c0 + z, 8), cs), :]))], axis=0)
        else:
            gu = dot_nt(get_xn(tm), b16(wgu_v[c0:c0 + cs, :]))
        if cs % 128 == 0:
            return geglu2(gu[:, :cs], gu[:, cs:]).astype(BF16), gu
        return geglu2(gu, pltpu.roll(gu, cs, 1))[:, :cs].astype(BF16), gu

    def down_chunk(ci, h):
        c0, cs = CHUNKS[ci]
        return dot_nn(h, b16(wd_v[c0 // 2:(c0 + cs) // 2, :]))

    def finish(tm, acc, b, prow):
        o = jnp.concatenate([a_scr[j, HALO:HALO + tm, :].astype(BF16) for j in range(NT)], axis=1)
        res = 0.5 * acc + dot_nn(o, b16(wop[...])) + b16(xx[prow, :]).astype(F32)
        res = u32(res.astype(BF16))
        if OUTSPLIT:
            for j in range(NT):
                out_v[prow, j * 128:(j + 1) * 128] = res[:, j * 128:(j + 1) * 128]
                out_copy(b, prow, j).start()
        else:
            out_v[prow, :] = res
            out_copy(b, prow, 0).start()

    def block0():
        tm = TM0
        hs = {}
        for h in range(2):
            wait(h)
            for r in range(h * tm // 2, (h + 1) * tm // 2, 32):
                xn_scr[r // 2:r // 2 + 16, :] = u32(ln_rows(r // 2, 32).astype(BF16))
        z = z_smem[0]
        wait(2)
        hs[0], _ = gu_chunk(tm, 0, z)
        wait(3)
        hs[1], _ = gu_chunk(tm, 1)
        wait(4)
        hs[2], _ = gu_chunk(tm, 2)
        prep_qkv(0)
        proj(tm, 0, 0, 4)
        wait(5)
        proj(tm, 0, 4, 5)
        hs[TAIL], _ = gu_chunk(tm, TAIL)
        hs[3], _ = gu_chunk(tm, 3)
        prep_qkv(1)
        proj(tm, 1)
        prep_qkv(2)
        proj(tm, 2)
        wait(6)
        att = Att(tm, True, z, 0, 0, SPAN0, TM0 // 2)
        prep_wo()
        for ci in (4, 5, 6):
            hs[ci], gu = gu_chunk(tm, ci)
            att.emit(gu, 5)
        wait(7)
        acc = None
        for ci in range(NCH):
            d = down_chunk(ci, hs[ci])
            acc = d if acc is None else acc + d
            att.emit(acc, -(-CHUNKS[ci][1] // 128))
        att.flush()
        publish_xn()
        finish(tm, acc, 0, pl.ds(0, TM0 // 2))

    def prow1(b):
        return pl.ds(pl.multiple_of(TM0 // 2 + (b - 1) * (TM1 // 2), 8), TM1 // 2)

    def block(b):
        tm = TM1
        z = z_smem[0]
        nsrc = pl.multiple_of(TM0 // 2 + jnp.minimum(b, NB1 - 1) * (TM1 // 2), 8)
        for p in range(3):
            proj(tm, p)
        att = Att(tm, False, z, 75, 75 + T0, SPAN, nsrc)
        hs = {}
        for ci in [TAIL] + list(range(TAIL)):
            hs[ci], gu = gu_chunk(tm, ci)
            att.emit(gu, 5)
        att.flush()
        publish_xn()
        h = jnp.concatenate([hs[ci] for ci in range(NCH)], axis=1)
        finish(tm, dot_nn(h, b16(wd_v[...])), b, prow1(b))

    for g in groups:
        for c in g:
            c.start()
    a_scr[NT:3 * NT, 0:HALO, :] = jnp.zeros((2 * NT, HALO, 128), F32)
    block0()

    def body(b, carry):
        block(b)
        return carry

    if not ONLY0:
        lax.fori_loop(1, NB1 + 1, body, 0)
    for b in range(1 if ONLY0 else NB1 + 1):
        for j in range(NT if OUTSPLIT else 1):
            out_copy(b, pl.ds(0, TM0 // 2) if b == 0 else prow1(b), j).wait()


@jax.jit
def pallas_parallel_sum__sliding_local_dilated__geglu_ffn__prompt_kernel(A_x, A_wqkv, A_wo, B_x, B_w_gate, B_w_up, B_w_down):
    x = A_x.reshape(S, D)
    hbm = pl.BlockSpec(memory_space=pl.ANY)
    out = pl.pallas_call(
        kernel,
        in_specs=[hbm] * 6,
        out_specs=hbm,
        out_shape=jax.ShapeDtypeStruct((S, D), BF16),
        scratch_shapes=[
            pltpu.VMEM((FEN + 8, D), U32),
            pltpu.VMEM((TM0 // 2, D), U32),
            pltpu.VMEM((D // 2, 3 * D), U32),
            pltpu.VMEM((D // 2, D), U32),
            pltpu.VMEM((F, D), U32),
            pltpu.VMEM((F // 2, D), U32),
            pltpu.VMEM((3 * D // 2, D), U32),
            pltpu.VMEM((D // 2, D), U32),
            pltpu.VMEM((3, NT, D, 128), F32),
            pltpu.VMEM((3 * NT + 1, TM0 + HALO, 128), F32),
            pltpu.VMEM((S // 2, D), U32),
            pltpu.SMEM((1,), jnp.int32),
            pltpu.SemaphoreType.DMA((2 * NCH + 8,)),
            pltpu.SemaphoreType.DMA(((NB1 + 1) * NT,)),
        ],
        compiler_params=pltpu.CompilerParams(vmem_limit_bytes=100 * 1024 * 1024),
    )(x, A_wqkv, A_wo, B_w_gate.T, B_w_up.T, B_w_down)
    return out.reshape(1, S, D)
```

```python
import functools
import math
import jax
import jax.numpy as jnp
from jax import lax
import jax.experimental.pallas as pl
import jax.experimental.pallas.tpu as pltpu

S, D, F, H, DH, W, DIL = 2048, 640, 1728, 32, 20, 8, 2
NT = D // 128
TM0 = 512
TM1 = 384
NB1 = (S - TM0) // TM1
XR = TM0 // NB1
HALO = 16
FM = 1664
FT = F - FM
QSCALE = DH ** -0.5 * math.log2(math.e)
NEG = -1e9 * DH ** 0.5
GELU_C1 = math.sqrt(2.0 / math.pi)
GELU_C2 = GELU_C1 * 0.044715
F32, BF16, U32 = jnp.float32, jnp.bfloat16, jnp.uint32
RA = 8
NBABY, NGIANT = 16, 4
PB = 4

SW = 2
SPAN = 112
SPAN0 = 120
LAG = 0
EXTRA0 = 36
XL = 2
LASTSPLIT = 2
T1E = 0
TA = 0
TW2 = 3
PUBT = 24
TPUB = 216
G1 = 15
P2 = 48
TS = 4
TG = 4
TE = -1
LINKD = 2
FULL = 4
BACKD = 48
COPYW = 1
G4 = 3
RL = 0
T4 = 20

CHUNKS = [(0, 128), (128, 256), (384, 128), (512, 384), (896, 256), (1152, 256), (1408, 256), (FM, FT)]
TAIL = len(CHUNKS) - 1


def dot_nn(a, b):
    return jnp.dot(a, b, preferred_element_type=F32)


def dot_nt(a, b):
    return lax.dot_general(a, b, (((1,), (1,)), ((), ())), preferred_element_type=F32)


def geglu2(g, u):
    inner = g * (GELU_C1 + GELU_C2 * (g * g))
    a = g * u
    return a + a * jnp.tanh(inner)


def b16(v):
    return pltpu.bitcast(v, BF16)


def u32(v):
    return pltpu.bitcast(v, U32)


def lanes(j):
    return slice(j * 128, (j + 1) * 128)


def store_packed(ref, rows, col0, v):
    for c in range(0, v.shape[1], 128):
        ref[rows, col0 + c:col0 + c + 128] = u32(v[:, c:c + 128].astype(BF16))


class Pacer:
    def __init__(self, tm, passes, tasks):
        self.tm, self.passes = tm, passes
        self.tasks = sorted(tasks, key=lambda t: t[0])

    def __call__(self, part, k):
        rnd = self.passes // 4
        self.passes += 1
        while k != 1 and self.tasks and self.tasks[0][0] < 4 * (rnd + 1):
            t, fn = self.tasks.pop(0)
            frac = max(0.0, (t - 4 * rnd) / 4)
            tr = min(self.tm - 8, int(frac * self.tm) // 8 * 8)
            fn(part[tr:tr + 8])


def kernel(x_hbm, wqkv_hbm, wo_hbm, wgt_hbm, wut_hbm, wd_hbm, out_hbm,
           x0_v, xq, wqkv_v, wo_v, wgu_v, wd_v, out0_v, out_v,
           xn_scr, nx_scr, wqkvp, wop, wgup, wdp, w0, h_scr,
           t_scr, a_scr, v_scr, g_scr, b_scr, r_scr, keep,
           g0_scr, z_smem, sem_i, sem_x, sem_o):
    z_smem[0] = 0

    def out_copy(buf, rows, cols):
        return pltpu.make_async_copy(buf.at[rows, cols], out_hbm.at[rows, cols], sem_o.at[0])

    def x_copy(lo, hi):
        return [(x_hbm.at[pl.ds(lo, hi - lo)], x0_v.at[pl.ds(lo, hi - lo)])]

    def x_block(b, slot):
        row = TM0 + min(b, NB1 - 1) * TM1 if isinstance(b, int) else pl.multiple_of(
            TM0 + jnp.minimum(b, NB1 - 1) * TM1, 16)
        return x_hbm.at[pl.ds(row, TM1)], xq.at[pl.ds(slot * TM1, TM1)]

    def x_refill(b, z):
        for slot in range(2):
            pltpu.make_async_copy(*x_block(b + 1 - slot, slot), sem_x.at[0]).start()
        return xq[pl.ds(pl.multiple_of(2 * TM1 + 16 + z, 16), 16), 0:128].astype(F32)

    def x_wait():
        for slot in range(2):
            pltpu.make_async_copy(*x_block(0, slot), sem_x.at[0]).wait()

    def gu_copy(ci):
        c0, cs = CHUNKS[ci]
        return [(wgt_hbm.at[pl.ds(c0, cs)], wgu_v.at[pl.ds(2 * c0, cs)]),
                (wut_hbm.at[pl.ds(c0, cs)], wgu_v.at[pl.ds(2 * c0 + cs, cs)])]

    def wqkv_copy(lo, hi):
        return [(wqkv_hbm.at[:, pl.ds(lo * D, (hi - lo) * D)], wqkv_v.at[:, pl.ds(lo * D, (hi - lo) * D)])]

    groups = [
        x_copy(0, TM0 // 2),
        x_copy(TM0 // 2, TM0),
        gu_copy(0),
        gu_copy(1),
        gu_copy(2) + gu_copy(TAIL) + wqkv_copy(0, 1),
        gu_copy(3) + wqkv_copy(1, 3),
        gu_copy(4) + gu_copy(5) + gu_copy(6) + [x_block(0, 0), (wo_hbm, wo_v), (wd_hbm, wd_v)],
    ]
    groups = [[pltpu.make_async_copy(src, dst, sem_i.at[g]) for src, dst in grp] for g, grp in enumerate(groups)]

    def wait(g):
        for c in groups[g]:
            c.wait()

    def fence_x(val8, z):
        xq[pl.ds(pl.multiple_of(2 * TM1 + z, 8), 8), 0:128] = val8.astype(BF16)

    def fence_n(val8, z):
        nx_scr[pl.ds(pl.multiple_of(TM1 // 2 + z, 8), 8), 0:128] = u32(val8)

    def fence_a(val8, z):
        a_scr[3 * NT, pl.ds(pl.multiple_of(z, 8), 8), :] = val8

    def fence_v(val8, z):
        v_scr[pl.ds(pl.multiple_of(FT * NT * 8 + z, 8), 8), :] = val8

    def fence_g(val8, z):
        g_scr[pl.ds(pl.multiple_of(XR + TM1 + z, 8), 8), :] = val8

    def ln_rows(r, n):
        x = x0_v[r:r + n, :].astype(F32)
        m = jnp.sum(x, axis=-1, keepdims=True) * (1.0 / D)
        xc = x - m
        var = jnp.sum(xc * xc, axis=-1, keepdims=True) * (1.0 / D)
        return xc * lax.rsqrt(var + 1e-5)

    def ln_x(src):
        return xq[src:src + 16, :].astype(F32)

    def ln_mean(src):
        return jnp.broadcast_to(jnp.sum(ln_x(src), axis=-1, keepdims=True) * (1.0 / D), (16, 128))

    def ln_rstd(src, m):
        xc = ln_x(src) - jnp.concatenate([m] * NT, axis=1)
        var = jnp.sum(xc * xc, axis=-1, keepdims=True) * (1.0 / D)
        return jnp.broadcast_to(lax.rsqrt(var + 1e-5), (16, 128))

    def ln_apply(src, c, m, rs):
        y = (ln_x(src) - jnp.concatenate([m] * NT, axis=1)) * jnp.concatenate([rs] * NT, axis=1)
        store_packed(nx_scr, pl.ds(c * 8, 8), 0, y)
        return y[:, 0:128]

    def prep_qkv(p):
        for c in range(NT):
            bt = wqkv_v[:, lanes(p * NT + c)].astype(F32).T
            for j in range(NT):
                t_scr[p, j, lanes(c), :] = bt[:, lanes(j)]
        for d in range(DH):
            for j in range(NT):
                rows = t_scr[p, j, pl.ds(d, H, stride=DH), :]
                wqkvp[(p * D + d * H) // 2:(p * D + (d + 1) * H) // 2, lanes(j)] = u32(rows.astype(BF16))

    def prep_wo():
        for j in range(NT):
            t_scr[0, j] = wo_v[:, lanes(j)].astype(F32)
            for d in range(DH):
                rows = t_scr[0, j, pl.ds(d, H, stride=DH), :]
                wop[d * H // 2:(d + 1) * H // 2, lanes(j)] = u32(rows.astype(BF16))

    def prep_table_pieces(z):
        def skew(j):
            def run():
                m = 0.5 * wd_v[FM:F, lanes(j)].astype(F32)
                lane = lax.broadcasted_iota(jnp.int32, (FT, 128), 1)
                for bit in range(6):
                    sh = 1 << bit
                    if sh % 8 == 0:
                        up = jnp.concatenate([m[sh:], m[:sh]], axis=0)
                    else:
                        t_scr[1, j, bit * 128:bit * 128 + FT, :] = m
                        t_scr[1, j, bit * 128 + FT:bit * 128 + FT + 8, :] = m[0:8]
                        up = t_scr[1, j, bit * 128 + sh:bit * 128 + sh + FT, :]
                    m = jnp.where((lane & sh) != 0, up, m)
                for a in range(NGIANT):
                    blk = m[a * NBABY:(a + 1) * NBABY]
                    t_scr[2, j, a * NBABY:(a + 1) * NBABY, :] = pltpu.roll(blk, a * NBABY, 1) if a else blk
                return jnp.sum(m.reshape(FT // 8, 8, 128), axis=0)
            return run

        def spread(j, a):
            def run():
                blk = t_scr[2, j, a * NBABY:(a + 1) * NBABY, :]
                for b in range(NBABY):
                    r0 = ((a * NBABY + b) * NT + j) * 8
                    v_scr[r0:r0 + 8, :] = jnp.broadcast_to(blk[b:b + 1], (8, 128))
                return v_scr[pl.ds(pl.multiple_of(z, 8), 8), :]
            return run

        return [skew(j) for j in range(NT)] + [spread(j, a) for j in range(NT) for a in range(NGIANT)]

    def gu_w(first, r0, n, cols=slice(None)):
        if not first and COPYW:
            return b16(wgup[r0 // 2:(r0 + n) // 2, cols])
        w = wgu_v[r0:r0 + n, cols]
        if COPYW:
            wgup[r0 // 2:(r0 + n) // 2, cols] = u32(w)
        return w

    def d_w(first, k, j):
        if not first and COPYW:
            return b16(wdp[k * 64:(k + 1) * 64, lanes(j)])
        w = wd_v[lanes(k), lanes(j)]
        if COPYW:
            wdp[k * 64:(k + 1) * 64, lanes(j)] = u32(w)
        return w

    def passes(n, dot, lhs, rhs, pace):
        y = None
        for k in range(n):
            part = dot(lhs(k), rhs(k))
            y = part if y is None else y + part
            pace(part, k)
        return y

    def xn_k(tm):
        return lambda k: b16(xn_scr[0:tm // 2, lanes(k)])

    def proj(tm, p, pace=None):
        if pace is None:
            y = dot_nt(b16(xn_scr[0:tm // 2, :]), b16(wqkvp[p * D // 2:(p + 1) * D // 2, :]))
        for j in range(NT):
            r0 = (p * NT + j) * 64
            a_scr[p * NT + j, HALO:HALO + tm, :] = y[:, lanes(j)] if pace is None else passes(
                NT, dot_nt, xn_k(tm), lambda k: b16(wqkvp[r0:r0 + 64, lanes(k)]), pace)

    def gu_chunk(tm, ci, first, pace=None, z=None):
        c0, cs = CHUNKS[ci]
        if pace is not None:
            for t in range(cs // 128):
                g, u = [passes(NT, dot_nt, xn_k(tm), lambda k: gu_w(first, r0, 128, lanes(k)), pace)
                        for r0 in (2 * c0 + t * 128, 2 * c0 + cs + t * 128)]
                store_packed(h_scr, pl.ds(0, tm // 2), c0 + t * 128, geglu2(g, u))
        elif ci == TAIL:
            g0_scr[...] = dot_nt(b16(xn_scr[0:tm // 2, :]), wgu_v[2 * c0:2 * c0 + 2 * cs, :])
        else:
            w = gu_w(first, 2 * c0, 2 * cs)
            if z is None:
                gu = dot_nt(b16(xn_scr[0:tm // 2, :]), w)
            else:
                gu = jnp.concatenate([
                    dot_nt(b16(xn_scr[0:tm // 4, :]), w),
                    dot_nt(b16(xn_scr[tm // 4:tm // 2, :]), wgu_v[pl.ds(pl.multiple_of(2 * c0 + z, 16), 2 * cs), :])],
                    axis=0)
            store_packed(h_scr, pl.ds(0, tm // 2), c0, geglu2(gu[:, :cs], gu[:, cs:]))

    def down(tm, first, pace):
        return [passes(FM // 128, dot_nn, lambda k: b16(h_scr[0:tm // 2, lanes(k)]), lambda k: d_w(first, k, j), pace)
                for j in range(NT)]

    def finish(tm, acc, pace, row0, x0=None):
        o = [b16(a_scr[3 * NT + 1 + k, 0:tm // 2, :]) for k in range(NT)]
        ys = []
        for j in range(NT + LAG):
            if j < NT:
                ys.append(passes(NT, dot_nn, lambda k: o[k], lambda k: b16(wop[k * 64:(k + 1) * 64, lanes(j)]), pace))
            k = j - LAG
            if k < 0:
                continue
            if x0 is None:
                keep[k] = 0.5 * acc[k] + x0_v[:, lanes(k)].astype(F32) + ys[k]
                continue
            n = tm // LASTSPLIT if k == NT - 1 else tm
            for r in range(0, tm, n):
                rows = pl.ds(pl.multiple_of(row0 + r, 16), n)
                res = 0.5 * acc[k][r:r + n] + r_scr[k, XR + r:XR + r + n, :]
                out_v[rows, lanes(k)] = (res + ys[k][r:r + n]).astype(BF16)
                if k == NT - 1 and r + n == tm:
                    out_copy(out0_v, pl.ds(pl.multiple_of(x0 + XR - 16 * G4, 16), 16 * G4), pl.ds(0, D)).start()
                out_copy(out_v, rows, pl.ds(k * 128, 128)).start()
        assert not pace.tasks

    def att_qk(first, r, z):
        q = a_scr[0:NT, HALO + r:HALO + r + RA, :]
        s = []
        for w in range(W):
            lo = HALO + r - DIL * w
            sw = jnp.sum(q * a_scr[NT:2 * NT, lo:lo + RA, :], axis=0)
            if (w + 1) % SW == 0:
                fence_a(sw, z)
            t = sw + pltpu.roll(sw, 64, 1)
            s.append(t + pltpu.roll(t, 32, 1))
        if first and r < DIL * (W - 1):
            pos = r + lax.broadcasted_iota(jnp.int32, (RA, 128), 0)
            s = [jnp.where(pos >= DIL * w, s[w], NEG) for w in range(W)]
        return s

    def att_pv(r, z, s):
        mx = functools.reduce(jnp.maximum, s)
        p = [jnp.exp2((l - mx) * QSCALE) for l in s]
        den = functools.reduce(lambda a, b: a + b, p)
        inv = pl.reciprocal(den, approx=True)
        inv = inv * (2.0 - den * inv)
        o = None
        for w in range(W):
            lo = HALO + r - DIL * w
            t = p[w][None] * a_scr[2 * NT:3 * NT, lo:lo + RA, :]
            o = t if o is None else o + t
            if (w + 1) % SW == 0 and w < W - 1:
                fence_a(o[NT - 1], z)
        o = o * inv[None]
        if r % 16 == 0:
            a_scr[0:NT, pl.ds(pl.multiple_of(HALO + r + z, 8), RA), :] = o
        else:
            both = jnp.concatenate([a_scr[0:NT, HALO + r - RA:HALO + r, :], o], axis=1)
            for j in range(NT):
                a_scr[3 * NT + 1 + j, pl.ds(pl.multiple_of((r - RA) // 2 + z, 8), 8), :] = pltpu.bitcast(
                    both[j].astype(BF16), F32)
        return o[0]

    def att_tasks(tm, first, z, t0, span, tpub, nb, extra, done=None, back=None):
        na = tm // RA
        nln = TM1 // 16
        n = max(na + 1, 2 * nln + 2)
        links, pend, m, rs = [], [], {}, {}

        def step(i):
            def run(trig):
                c = i // 2
                fence_a(trig, z)
                if c <= nln:
                    fence_x(trig, z)
                for _, v in [l for l in links if l[0] <= i]:
                    for r in range(0, v.shape[0], 8):
                        fence_a(v[r:r + 8], z)
                links[:] = [l for l in links if l[0] > i]
                if done:
                    links.append((i + 1, done[-1]))
                    done.clear()
                if i % 2 == 0:
                    if c < nln:
                        m[c] = ln_mean(c * 16)
                        links.append((i + 1, m[c]))
                else:
                    if 0 < c <= nln:
                        links.append((i + 1, ln_apply((c - 1) * 16, c - 1, m[c - 1], rs[c - 1])))
                    if c == nln:
                        links.append((i + 1, x_refill(nb, z)))
                    if c < nln:
                        rs[c] = ln_rstd(c * 16, m[c])
                        links.append((i + 2, rs[c]))
                if i in extra:
                    links.append((i + XL, extra.pop(i)()))
                if i < na:
                    pend.append(att_qk(first, i * RA, z))
                if 1 <= i <= na:
                    last = att_pv((i - 1) * RA, z, pend.pop(0))
                    if back is not None:
                        back[:] = [last]
                if i == n - 1:
                    assert not extra
                    for _, v in links:
                        if back is not None:
                            back[0] = back[0] + v[0:8] + v[v.shape[0] - 8:]
                    a_scr[NT:3 * NT, 0:HALO, :] = a_scr[NT:3 * NT, tm:tm + HALO, :]
            return run

        def publish(c):
            def run(trig):
                fence_n(trig, z)
                xn_scr[c * 8:(c + 1) * 8, :] = nx_scr[c * 8:(c + 1) * 8, :]
            return run

        tasks = [(t0 + span * i / n, step(i)) for i in range(n)]
        t = tpub
        for c in range(nln):
            t = max(t, t0 + span * (2 * c + 4.5) / n)
            tasks.append((t, publish(c)))
            t += PUBT / 10
        return tasks

    def tail_tasks(z, b, wins, done, back):
        x0 = pl.multiple_of(b * XR, 16)
        g_scr[0:XR, :] = g0_scr[pl.ds(x0, XR), :]
        r_scr[:, 0:XR, :] = keep[:, pl.ds(x0, XR), :]
        times = []
        for lo, hi, num in wins:
            times += [lo + (hi - lo) * i / num for i in range(num)]
        npc = FT // PB
        assert len(times) == (XR + TM1) // 16 * npc
        st = dict(acc=None, tot=None, n=0)
        links = []

        def rolls(g):
            def run(trig):
                if trig is not None:
                    fence_g(trig, z)
                gu = g_scr[g * 16:(g + 1) * 16, :]
                ru = pltpu.roll(gu, FT, 1)
                low = lax.broadcasted_iota(jnp.int32, gu.shape, 1) < FT
                hh = geglu2(jnp.where(low, gu, ru), jnp.where(low, ru, gu))
                b_scr[0, g * 16:(g + 1) * 16, :] = hh
                for i in range(1, NBABY):
                    b_scr[i, g * 16:(g + 1) * 16, :] = pltpu.roll(hh, 128 - i, 1)
            return run

        def piece(g, s0):
            def run(trig):
                st["n"] += 1
                if back and s0 == 0:
                    links.append((st["n"] + BACKD // PB, back.pop()))
                for _, v in [l for l in links if l[0] <= st["n"]]:
                    trig = trig + v
                links[:] = [l for l in links if l[0] > st["n"]]
                fence_v(trig, z)
                for s in range(s0, s0 + PB):
                    a, i = divmod(s, NBABY)
                    rb = b_scr[i, g * 16:(g + 1) * 16, :].reshape(1, 2, 8, 128)
                    t = rb * v_scr[s * NT * 8:(s + 1) * NT * 8, :].reshape(NT, 1, 8, 128)
                    st["acc"] = t if i == 0 else st["acc"] + t
                    if i == NBABY - 1:
                        acc = st["acc"].reshape(NT * 16, 128)
                        st["tot"] = acc if a == 0 else st["tot"] + pltpu.roll(acc, 128 - a * NBABY, 1)
                if (s0 + PB) % FULL == 0:
                    v = jnp.sum(st["acc"].reshape(2 * NT, 8, 128), axis=0)
                    links.append((st["n"] + LINKD, v))
                    done.append(v)
                else:
                    k = st["n"] % (2 * NT)
                    links.append((st["n"] + LINKD, st["acc"][k // 2, k % 2]))
                if s0 + PB == FT:
                    tot = st["tot"].reshape(NT, 16, 128)
                    if g < XR // 16:
                        rows = pl.ds(pl.multiple_of(x0 + g * 16, 16), 16)
                        tot = tot + r_scr[:, g * 16:(g + 1) * 16, :]
                        out0_v[rows, :] = jnp.concatenate([tot[j] for j in range(NT)], axis=1).astype(BF16)
                        if g == XR // 16 - G4 - 1:
                            out_copy(out0_v, pl.ds(pl.multiple_of(x0, 16), XR - 16 * G4), pl.ds(0, D)).start()
                    else:
                        if st["n"] > G1 * npc:
                            tot = tot + r_scr[:, g * 16:(g + 1) * 16, :]
                        r_scr[:, g * 16:(g + 1) * 16, :] = tot
                    links.append((st["n"] + 32 // PB, jnp.sum(tot.reshape(2 * NT, 8, 128), axis=0)))
            return run

        nx = XR // 16
        order = list(range(nx - G4)) + list(range(nx, nx + TM1 // 16)) + list(range(nx - G4, nx))
        rolls(order[0])(None)
        tasks = []
        for q, g in enumerate(order):
            if q:
                tasks.append((times[(q - 1) * npc] + 0.01, rolls(g)))
            for i in range(npc):
                tasks.append((times[q * npc + i], piece(g, i * PB)))
        return tasks

    def residual(c):
        def run():
            x = xq[TM1 + c * 16:TM1 + (c + 1) * 16, :].astype(F32)
            x = jnp.stack([x[:, lanes(j)] for j in range(NT)])
            rows = slice(XR + c * 16, XR + (c + 1) * 16)
            if c < G1 - (XR // 16 - G4):
                x = x + r_scr[:, rows, :]
            r_scr[:, rows, :] = x
            return jnp.sum(x.reshape(2 * NT, 8, 128), axis=0) if RL else x[NT - 1]
        return run

    def block0():
        tm = TM0
        for h in range(2):
            if h:
                wait(h)
            for r in range(h * tm // 2, (h + 1) * tm // 2, 32):
                store_packed(xn_scr, pl.ds(r // 2, 16), 0, ln_rows(r, 32))
        z = z_smem[0]
        wait(2)
        gu_chunk(tm, 0, True, z=z)
        wait(3)
        gu_chunk(tm, 1, True)
        wait(4)
        gu_chunk(tm, TAIL, True)
        gu_chunk(tm, 2, True)
        prep_qkv(0)
        proj(tm, 0)
        w0[...] = u32(wgu_v[2 * FM:2 * F, :].astype(F32).T.astype(BF16))
        wait(5)
        gu_chunk(tm, 3, True)
        prep_qkv(1)
        proj(tm, 1)
        prep_qkv(2)
        proj(tm, 2)

        def last_region(i, carry):
            wait(6)
            pace = Pacer(tm, 2, att_tasks(tm, True, z, 2, SPAN0, 69, 0, dict(enumerate(prep_table_pieces(z), EXTRA0))))
            prep_wo()
            for ci in (4, 5, 6):
                gu_chunk(tm, ci, True, pace)
            finish(tm, down(tm, True, pace), pace, 0)
            return carry

        lax.fori_loop(0, z + 1, last_region, 0)

    def block(b, carry):
        tm = TM1
        x_wait()
        z = z_smem[0]
        x0 = b * XR
        tq, tg, td = 80, 210, 275
        done, back = [], []
        tasks = att_tasks(tm, False, z, tq + TA, SPAN, TPUB, b + 1,
                          {2 * c: residual(TM1 // 16 - 1 - c) for c in range(TM1 // 16)}, done, back)
        npc = FT // PB
        wins = [(TS, tq - T1E, G1 * npc), (tq + TA + SPAN + TW2, tg + TG, P2),
                (tg + TG, td - TE, ((XR + TM1) // 16 - G1 - G4) * npc - P2), (td - TE, td + T4, G4 * npc)]
        tasks += tail_tasks(z, b, wins, done, back)
        pace = Pacer(tm, 0, tasks)
        g_scr[XR:XR + tm, :] = passes(NT, dot_nn, xn_k(tm), lambda k: b16(w0[k * 64:(k + 1) * 64, :]), pace)
        for p in range(3):
            proj(tm, p, pace)
        for ci in range(TAIL):
            gu_chunk(tm, ci, False, pace)
        finish(tm, down(tm, False, pace), pace, TM0 + b * TM1, x0)
        return carry

    def body(b, carry):
        return block(b, carry)

    def outer(i, carry):
        block0()
        return lax.fori_loop(0, NB1, body, carry)

    for g in groups:
        for c in g:
            c.start()
    xq[2 * TM1 + 16:, 0:128] = jnp.zeros((16, 128), BF16)
    a_scr[NT:3 * NT, 0:HALO, :] = jnp.zeros((2 * NT, HALO, 128), F32)
    wait(0)
    lax.fori_loop(0, z_smem[0] + 1, outer, 0)
    x_wait()
    out_copy(out0_v, pl.ds(0, TM0), pl.ds(0, D)).wait()
    out_copy(out_v, pl.ds(TM0, S - TM0), pl.ds(0, D)).wait()


@jax.jit
def pallas_parallel_sum__sliding_local_dilated__geglu_ffn__prompt_kernel(
        A_x, A_wqkv, A_wo, B_x, B_w_gate, B_w_up, B_w_down):
    hbm = pl.BlockSpec(memory_space=pl.ANY)
    out = pl.pallas_call(
        kernel,
        in_specs=[hbm] * 6,
        out_specs=hbm,
        out_shape=jax.ShapeDtypeStruct((S, D), BF16),
        scratch_shapes=[
            pltpu.VMEM((TM0, D), BF16),
            pltpu.VMEM((2 * TM1 + 32, D), BF16),
            pltpu.VMEM((D, 3 * D), BF16),
            pltpu.VMEM((D, D), BF16),
            pltpu.VMEM((2 * F, D), BF16),
            pltpu.VMEM((F, D), BF16),
            pltpu.VMEM((TM0, D), BF16),
            pltpu.VMEM((S, D), BF16),
            pltpu.VMEM((TM0 // 2, D), U32),
            pltpu.VMEM((TM1 // 2 + 8, D), U32),
            pltpu.VMEM((3 * D // 2, D), U32),
            pltpu.VMEM((D // 2, D), U32),
            pltpu.VMEM((FM, D), U32),
            pltpu.VMEM((FM // 2, D), U32),
            pltpu.VMEM((D // 2, 128), U32),
            pltpu.VMEM((TM0 // 2, FM), U32),
            pltpu.VMEM((3, NT, D, 128), F32),
            pltpu.VMEM((4 * NT + 1, TM0 + HALO, 128), F32),
            pltpu.VMEM((FT * NT * 8 + 8, 128), F32),
            pltpu.VMEM((XR + TM1 + 8, 128), F32),
            pltpu.VMEM((NBABY, XR + TM1, 128), F32),
            pltpu.VMEM((NT, XR + TM1, 128), F32),
            pltpu.VMEM((NT, TM0, 128), F32),
            pltpu.VMEM((TM0, 128), F32),
            pltpu.SMEM((1,), jnp.int32),
            pltpu.SemaphoreType.DMA((7,)),
            pltpu.SemaphoreType.DMA((1,)),
            pltpu.SemaphoreType.DMA((1,)),
        ],
        compiler_params=pltpu.CompilerParams(
            vmem_limit_bytes=100 * 1024 * 1024, disable_bounds_checks=True, disable_semaphore_checks=True),
    )(A_x.reshape(S, D), A_wqkv, A_wo, B_w_gate.T, B_w_up.T, B_w_down)
    return out.reshape(1, S, D)
```

```python
import functools
import math
import jax
import jax.numpy as jnp
from jax import lax
import jax.experimental.pallas as pl
import jax.experimental.pallas.tpu as pltpu

S, D, F, H, DH, W, DIL = 2048, 640, 1728, 32, 20, 8, 2
NT = D // 128
TM0 = 512
TM1 = 384
NB1 = (S - TM0) // TM1
XR = TM0 // NB1
HALO = 16
FM = 1664
FT = F - FM
QSCALE = DH ** -0.5 * math.log2(math.e)
NEG = -1e9 * DH ** 0.5
GELU_C1 = math.sqrt(2.0 / math.pi)
GELU_C2 = GELU_C1 * 0.044715
F32, BF16, U32 = jnp.float32, jnp.bfloat16, jnp.uint32
RA = 8
NBABY, NGIANT = 16, 4
PB = 4

SW = 2
T00 = 4
SPAN0 = 120
EXTRA0 = 40
TP0 = 72
PUBT0 = 20
SPAN = 112
TPUB = 216
PUBT = 23
TS = 4
G1 = 15
TW2 = 0
P2 = 48
TG = 2
G4 = 3
TE = 0
T4 = 20
BACKD = 14

CHUNKS = [(0, 128), (128, 256), (384, 128), (512, 384), (896, 256), (1152, 256), (1408, 256), (FM, FT)]
TAIL = len(CHUNKS) - 1


def dot_nn(a, b):
    return jnp.dot(a, b, preferred_element_type=F32)


def dot_nt(a, b):
    return lax.dot_general(a, b, (((1,), (1,)), ((), ())), preferred_element_type=F32)


def geglu2(g, u):
    inner = g * (GELU_C1 + GELU_C2 * (g * g))
    a = g * u
    return a + a * jnp.tanh(inner)


def b16(v):
    return pltpu.bitcast(v, BF16)


def u32(v):
    return pltpu.bitcast(v, U32)


def lanes(j):
    return slice(j * 128, (j + 1) * 128)


def store_packed(ref, rows, col0, v):
    for c in range(0, v.shape[1], 128):
        ref[rows, col0 + c:col0 + c + 128] = u32(v[:, c:c + 128].astype(BF16))


class Pacer:
    def __init__(self, tm, passes, tasks):
        self.tm, self.passes = tm, passes
        self.tasks = sorted(tasks, key=lambda t: t[0])

    def __call__(self, part, k):
        rnd = self.passes // 4
        self.passes += 1
        while k != 1 and self.tasks and self.tasks[0][0] < 4 * (rnd + 1):
            t, fn = self.tasks.pop(0)
            frac = max(0.0, (t - 4 * rnd) / 4)
            tr = min(self.tm - 8, int(frac * self.tm) // 8 * 8)
            fn(part[tr:tr + 8])


def kernel(x_hbm, wqkv_hbm, wo_hbm, wgt_hbm, wut_hbm, wd_hbm, out_hbm,
           x0_v, xq, wqkv_v, wo_v, wgu_v, wd_v, out0_v, out_v,
           u_scr, xn_scr, nx_scr, wqkvp, wop, wgup, wdp, w0, h_scr,
           t_scr, a_scr, v_scr, g_scr, b_scr, r_scr, keep,
           g0_scr, z_smem, sem_i, sem_x, sem_o):
    z_smem[0] = 0

    def out_copy(buf, rows, cols):
        return pltpu.make_async_copy(buf.at[rows, cols], out_hbm.at[rows, cols], sem_o.at[0])

    def x_copy(lo, hi):
        return [(x_hbm.at[pl.ds(lo, hi - lo)], x0_v.at[pl.ds(lo, hi - lo)])]

    def x_block(b, slot):
        row = TM0 + min(b, NB1 - 1) * TM1 if isinstance(b, int) else pl.multiple_of(
            TM0 + jnp.minimum(b, NB1 - 1) * TM1, 16)
        return x_hbm.at[pl.ds(row, TM1)], xq.at[pl.ds(slot * TM1, TM1)]

    def x_refill(b, z):
        for slot in range(2):
            pltpu.make_async_copy(*x_block(b + 1 - slot, slot), sem_x.at[0]).start()
        return xq[pl.ds(pl.multiple_of(2 * TM1 + 16 + z, 16), 16), 0:128].astype(F32)

    def x_wait():
        for slot in range(2):
            pltpu.make_async_copy(*x_block(0, slot), sem_x.at[0]).wait()

    def gu_copy(ci):
        c0, cs = CHUNKS[ci]
        return [(wgt_hbm.at[pl.ds(c0, cs)], wgu_v.at[pl.ds(2 * c0, cs)]),
                (wut_hbm.at[pl.ds(c0, cs)], wgu_v.at[pl.ds(2 * c0 + cs, cs)])]

    def wqkv_copy(lo, hi):
        return [(wqkv_hbm.at[:, pl.ds(lo * D, (hi - lo) * D)], wqkv_v.at[:, pl.ds(lo * D, (hi - lo) * D)])]

    groups = [
        x_copy(0, TM0 // 2),
        x_copy(TM0 // 2, TM0),
        gu_copy(0),
        gu_copy(1),
        gu_copy(2) + gu_copy(TAIL) + wqkv_copy(0, 1),
        gu_copy(3) + wqkv_copy(1, 3),
        gu_copy(4) + gu_copy(5) + gu_copy(6) + [x_block(0, 0), (wo_hbm, wo_v), (wd_hbm, wd_v)],
    ]
    groups = [[pltpu.make_async_copy(src, dst, sem_i.at[g]) for src, dst in grp] for g, grp in enumerate(groups)]

    def wait(g):
        for c in groups[g]:
            c.wait()

    def fence_x(val8, z):
        xq[pl.ds(pl.multiple_of(2 * TM1 + z, 8), 8), 0:128] = val8.astype(BF16)

    def fence_n(val8, z):
        nx_scr[pl.ds(pl.multiple_of(TM1 // 2 + z, 8), 8), 0:128] = u32(val8)

    def fence_a(val8, z):
        a_scr[3 * NT, pl.ds(pl.multiple_of(z, 8), 8), :] = val8

    def fence_v(val8, z):
        v_scr[pl.ds(pl.multiple_of(FT * NT * 8 + z, 8), 8), :] = val8

    def fence_g(val8, z):
        g_scr[pl.ds(pl.multiple_of(XR + TM1 + z, 8), 8), :] = val8

    def rnd(v):
        return v.astype(BF16).astype(F32)

    def wide(v):
        return jnp.concatenate([v] * NT, axis=1)

    def ln_mean(x):
        m = jnp.broadcast_to(jnp.sum(x, axis=-1, keepdims=True) * (1.0 / D), (x.shape[0], 128))
        mb = rnd(m)
        return mb, (m - mb) * (m - mb)

    def ln_rstd(xc, dd):
        var = jnp.broadcast_to(jnp.sum(xc * xc, axis=-1, keepdims=True) * (1.0 / D), dd.shape) - dd
        v = rnd(rnd(jnp.maximum(var, 0.0)) + 1e-5)
        std = rnd(v * lax.rsqrt(v))
        inv = pl.reciprocal(std, approx=True)
        return inv * (2.0 - std * inv)

    def ln_rows(r, n):
        x = x0_v[r:r + n, :].astype(F32)
        mb, dd = ln_mean(x)
        xc = x - wide(mb)
        return rnd(xc) * wide(ln_rstd(xc, dd))

    def ln_x(c):
        return xq[c * 16:(c + 1) * 16, :].astype(F32)

    def ln_apply(c, m, rs):
        y = rnd(ln_x(c) - wide(m)) * wide(rs)
        store_packed(nx_scr, pl.ds(c * 8, 8), 0, y)
        return y[:, 0:128]

    def prep_qkv(p):
        for c in range(NT):
            bt = wqkv_v[:, lanes(p * NT + c)].astype(F32).T
            for j in range(NT):
                t_scr[p, j, lanes(c), :] = bt[:, lanes(j)]
        for d in range(DH):
            for j in range(NT):
                rows = t_scr[p, j, pl.ds(d, H, stride=DH), :]
                wqkvp[(p * D + d * H) // 2:(p * D + (d + 1) * H) // 2, lanes(j)] = u32(rows.astype(BF16))

    def prep_wo():
        for j in range(NT):
            u_scr[j] = u32(wo_v[:, lanes(j)])
            for e in range(DH // 2):
                a = u_scr[j, pl.ds(e, H // 2, stride=DH), :]
                b = u_scr[j, pl.ds(DH // 2 + e, H // 2, stride=DH), :]
                wop[e * H:e * H + H // 2, lanes(j)] = (a & U32(0xFFFF)) | (b << 16)
                wop[e * H + H // 2:(e + 1) * H, lanes(j)] = (a >> 16) | (b & U32(0xFFFF0000))

    def prep_table_pieces(z):
        def skew(j):
            def run():
                m = 0.5 * wd_v[FM:F, lanes(j)].astype(F32)
                lane = lax.broadcasted_iota(jnp.int32, (FT, 128), 1)
                for bit in range(6):
                    sh = 1 << bit
                    up = jnp.concatenate([m[sh:], m[:sh]], axis=0) if sh % 8 == 0 else pltpu.roll(m, FT - sh, 0)
                    m = jnp.where((lane & sh) != 0, up, m)
                for a in range(NGIANT):
                    blk = m[a * NBABY:(a + 1) * NBABY]
                    t_scr[2, j, a * NBABY:(a + 1) * NBABY, :] = pltpu.roll(blk, a * NBABY, 1) if a else blk
                return jnp.sum(m.reshape(FT // 8, 8, 128), axis=0)
            return run

        def spread(j, a):
            def run():
                blk = t_scr[2, j, a * NBABY:(a + 1) * NBABY, :]
                for b in range(NBABY):
                    r0 = ((a * NBABY + b) * NT + j) * 8
                    v_scr[r0:r0 + 8, :] = jnp.broadcast_to(blk[b:b + 1], (8, 128))
                return v_scr[pl.ds(pl.multiple_of(z, 8), 8), :]
            return run

        return [skew(j) for j in range(NT)] + [spread(j, a) for j in range(NT) for a in range(NGIANT)]

    def gu_w(first, r0, n, cols=slice(None)):
        if not first:
            return b16(wgup[r0 // 2:(r0 + n) // 2, cols])
        w = wgu_v[r0:r0 + n, cols]
        wgup[r0 // 2:(r0 + n) // 2, cols] = u32(w)
        return w

    def d_w(first, k, j):
        if not first:
            return b16(wdp[k * 64:(k + 1) * 64, lanes(j)])
        w = wd_v[lanes(k), lanes(j)]
        wdp[k * 64:(k + 1) * 64, lanes(j)] = u32(w)
        return w

    def passes(n, dot, lhs, rhs, pace, y=None, k0=0):
        for k in range(k0, n):
            part = dot(lhs(k), rhs(k))
            y = part if y is None else y + part
            pace(part, k)
        return y

    def xn_k(tm):
        return lambda k: b16(xn_scr[0:tm // 2, lanes(k)])

    def proj(tm, p, pace=None):
        if pace is None:
            y = dot_nt(b16(xn_scr[0:tm // 2, :]), b16(wqkvp[p * D // 2:(p + 1) * D // 2, :]))
        for j in range(NT):
            r0 = (p * NT + j) * 64
            a_scr[p * NT + j, HALO:HALO + tm, :] = y[:, lanes(j)] if pace is None else passes(
                NT, dot_nt, xn_k(tm), lambda k: b16(wqkvp[r0:r0 + 64, lanes(k)]), pace)

    def gu_chunk(tm, ci, first, pace=None, z=None):
        c0, cs = CHUNKS[ci]
        if pace is not None:
            for t in range(cs // 128):
                g, u = [passes(NT, dot_nt, xn_k(tm), lambda k: gu_w(first, r0, 128, lanes(k)), pace)
                        for r0 in (2 * c0 + t * 128, 2 * c0 + cs + t * 128)]
                store_packed(h_scr, pl.ds(0, tm // 2), c0 + t * 128, geglu2(g, u))
        elif ci == TAIL:
            g0_scr[...] = dot_nt(b16(xn_scr[0:tm // 2, :]), wgu_v[2 * c0:2 * c0 + 2 * cs, :])
        else:
            w = gu_w(first, 2 * c0, 2 * cs)
            if z is None:
                gu = dot_nt(b16(xn_scr[0:tm // 2, :]), w)
            else:
                gu = jnp.concatenate([
                    dot_nt(b16(xn_scr[0:tm // 4, :]), w),
                    dot_nt(b16(xn_scr[tm // 4:tm // 2, :]), wgu_v[pl.ds(pl.multiple_of(2 * c0 + z, 16), 2 * cs), :])],
                    axis=0)
            store_packed(h_scr, pl.ds(0, tm // 2), c0, geglu2(gu[:, :cs], gu[:, cs:]))

    def h_k(tm):
        return lambda k: b16(h_scr[0:tm // 2, lanes(k)])

    def down(tm, first, pace, head=None):
        return [passes(FM // 128, dot_nn, h_k(tm), lambda k: d_w(first, k, j), pace,
                       *((head, 2) if j == 0 and head is not None else ()))
                for j in range(NT)]

    def finish(tm, acc, pace, row0=None, x0=None):
        o = [b16(a_scr[3 * NT + 1 + k, 0:tm // 2, :]) for k in range(NT)]
        for j in range(NT):
            y = passes(NT, dot_nn, lambda k: o[k], lambda k: b16(wop[k * 64:(k + 1) * 64, lanes(j)]), pace)
            if row0 is None:
                keep[j] = 0.5 * acc[j] + x0_v[:, lanes(j)].astype(F32) + y
                continue
            n = tm // 2 if j == NT - 1 else tm
            for r in range(0, tm, n):
                rows = pl.ds(pl.multiple_of(row0 + r, 16), n)
                res = 0.5 * acc[j][r:r + n] + r_scr[j, XR + r:XR + r + n, :]
                out_v[rows, lanes(j)] = (res + y[r:r + n]).astype(BF16)
                if j == NT - 1 and r + n == tm:
                    out_copy(out0_v, pl.ds(pl.multiple_of(x0 + XR - 16 * G4, 16), 16 * G4), pl.ds(0, D)).start()
                out_copy(out_v, rows, pl.ds(j * 128, 128)).start()
        assert not pace.tasks

    def att_qk(first, r, z):
        q = a_scr[0:NT, HALO + r:HALO + r + RA, :]
        s = []
        for w in range(W):
            lo = HALO + r - DIL * w
            sw = jnp.sum(q * a_scr[NT:2 * NT, lo:lo + RA, :], axis=0)
            if (w + 1) % SW == 0:
                fence_a(sw, z)
            t = sw + pltpu.roll(sw, 64, 1)
            s.append(t + pltpu.roll(t, 32, 1))
        if first and r < DIL * (W - 1):
            pos = r + lax.broadcasted_iota(jnp.int32, (RA, 128), 0)
            s = [jnp.where(pos >= DIL * w, s[w], NEG) for w in range(W)]
        return s

    def att_pv(r, z, s):
        mx = functools.reduce(jnp.maximum, s)
        p = [jnp.exp2((l - mx) * QSCALE) for l in s]
        den = functools.reduce(lambda a, b: a + b, p)
        inv = pl.reciprocal(den, approx=True)
        inv = inv * (2.0 - den * inv)
        o = None
        for w in range(W):
            lo = HALO + r - DIL * w
            t = p[w][None] * a_scr[2 * NT:3 * NT, lo:lo + RA, :]
            o = t if o is None else o + t
            if (w + 1) % SW == 0 and w < W - 1:
                fence_a(o[NT - 1], z)
        o = o * inv[None]
        if r % 16 == 0:
            a_scr[0:NT, pl.ds(pl.multiple_of(HALO + r + z, 8), RA), :] = o
        else:
            both = jnp.concatenate([a_scr[0:NT, HALO + r - RA:HALO + r, :], o], axis=1)
            for j in range(NT):
                a_scr[3 * NT + 1 + j, pl.ds(pl.multiple_of((r - RA) // 2 + z, 8), 8), :] = pltpu.bitcast(
                    both[j].astype(BF16), F32)
        return o[0]

    def att_tasks(tm, first, z, t0, span, tpub, nb, extra, done=None, back=None):
        na = tm // RA
        nln = TM1 // 16
        n = max(na + 1, 2 * nln + 2)
        links, pend, m, dd, rs = [], [], {}, {}, {}

        def step(i):
            def run(trig):
                c = i // 2
                fence_a(trig, z)
                if c <= nln:
                    fence_x(trig, z)
                for _, v in [l for l in links if l[0] <= i]:
                    for r in range(0, v.shape[0], 8):
                        fence_a(v[r:r + 8], z)
                links[:] = [l for l in links if l[0] > i]
                if done:
                    links.append((i + 1, done[-1]))
                    done.clear()
                if i % 2 == 0:
                    if c < nln:
                        m[c], dd[c] = ln_mean(ln_x(c))
                        links.append((i + 1, m[c]))
                else:
                    if 0 < c <= nln:
                        links.append((i + 1, ln_apply(c - 1, m[c - 1], rs[c - 1])))
                    if c == nln:
                        links.append((i + 1, x_refill(nb, z)))
                    if c < nln:
                        rs[c] = ln_rstd(ln_x(c) - wide(m[c]), dd[c])
                        links.append((i + 2, rs[c]))
                if i in extra:
                    links.append((i + 2, extra.pop(i)()))
                if i < na:
                    pend.append(att_qk(first, i * RA, z))
                if 1 <= i <= na:
                    last = att_pv((i - 1) * RA, z, pend.pop(0))
                    if back is not None:
                        back[:] = [last]
                if i == n - 1:
                    assert not extra
                    for _, v in links:
                        if back is not None:
                            back[0] = back[0] + v[0:8] + v[v.shape[0] - 8:]
                    a_scr[NT:3 * NT, 0:HALO, :] = a_scr[NT:3 * NT, tm:tm + HALO, :]
            return run

        def publish(c):
            def run(trig):
                fence_n(trig, z)
                xn_scr[c * 8:(c + 1) * 8, :] = nx_scr[c * 8:(c + 1) * 8, :]
            return run

        tasks = [(t0 + span * i / n, step(i)) for i in range(n)]
        t = tpub
        for c in range(nln):
            t = max(t, t0 + span * (2 * c + 4.5) / n)
            tasks.append((t, publish(c)))
            t += (PUBT0 if first else PUBT) / 10
        return tasks

    def tail_tasks(z, b, wins, done, back):
        x0 = pl.multiple_of(b * XR, 16)
        g_scr[0:XR, :] = g0_scr[pl.ds(x0, XR), :]
        r_scr[:, 0:XR, :] = keep[:, pl.ds(x0, XR), :]
        times = []
        for lo, hi, num in wins:
            times += [lo + (hi - lo) * i / num for i in range(num)]
        npc = FT // PB
        assert len(times) == (XR + TM1) // 16 * npc
        st = dict(acc=None, tot=None, n=0)
        links = []

        def rolls(g):
            def run(trig):
                if trig is not None:
                    fence_g(trig, z)
                gu = g_scr[g * 16:(g + 1) * 16, :]
                ru = pltpu.roll(gu, FT, 1)
                low = lax.broadcasted_iota(jnp.int32, gu.shape, 1) < FT
                hh = geglu2(jnp.where(low, gu, ru), jnp.where(low, ru, gu))
                b_scr[0, g * 16:(g + 1) * 16, :] = hh
                for i in range(1, NBABY):
                    b_scr[i, g * 16:(g + 1) * 16, :] = pltpu.roll(hh, 128 - i, 1)
            return run

        def piece(g, s0):
            def run(trig):
                st["n"] += 1
                if back and s0 == 0:
                    links.append((st["n"] + BACKD, back.pop()))
                for _, v in [l for l in links if l[0] <= st["n"]]:
                    trig = trig + v
                links[:] = [l for l in links if l[0] > st["n"]]
                fence_v(trig, z)
                for s in range(s0, s0 + PB):
                    a, i = divmod(s, NBABY)
                    rb = b_scr[i, g * 16:(g + 1) * 16, :].reshape(1, 2, 8, 128)
                    t = rb * v_scr[s * NT * 8:(s + 1) * NT * 8, :].reshape(NT, 1, 8, 128)
                    st["acc"] = t if i == 0 else st["acc"] + t
                    if i == NBABY - 1:
                        acc = st["acc"].reshape(NT * 16, 128)
                        st["tot"] = acc if a == 0 else st["tot"] + pltpu.roll(acc, 128 - a * NBABY, 1)
                v = jnp.sum(st["acc"].reshape(2 * NT, 8, 128), axis=0)
                links.append((st["n"] + 2, v))
                done.append(v)
                if s0 + PB == FT:
                    tot = st["tot"].reshape(NT, 16, 128)
                    if g < XR // 16:
                        rows = pl.ds(pl.multiple_of(x0 + g * 16, 16), 16)
                        tot = tot + r_scr[:, g * 16:(g + 1) * 16, :]
                        out0_v[rows, :] = jnp.concatenate([tot[j] for j in range(NT)], axis=1).astype(BF16)
                        if g == XR // 16 - G4 - 1:
                            out_copy(out0_v, pl.ds(pl.multiple_of(x0, 16), XR - 16 * G4), pl.ds(0, D)).start()
                    else:
                        if st["n"] > G1 * npc:
                            tot = tot + r_scr[:, g * 16:(g + 1) * 16, :]
                        r_scr[:, g * 16:(g + 1) * 16, :] = tot
                    links.append((st["n"] + 8, jnp.sum(tot.reshape(2 * NT, 8, 128), axis=0)))
            return run

        nx = XR // 16
        order = list(range(nx - G4)) + list(range(nx, nx + TM1 // 16)) + list(range(nx - G4, nx))
        rolls(order[0])(None)
        tasks = []
        for q, g in enumerate(order):
            if q:
                tasks.append((times[(q - 1) * npc] + 0.01, rolls(g)))
            for i in range(npc):
                tasks.append((times[q * npc + i], piece(g, i * PB)))
        return tasks

    def residual(c):
        def run():
            x = xq[TM1 + c * 16:TM1 + (c + 1) * 16, :].astype(F32)
            x = jnp.stack([x[:, lanes(j)] for j in range(NT)])
            rows = slice(XR + c * 16, XR + (c + 1) * 16)
            if c < G1 - (XR // 16 - G4):
                x = x + r_scr[:, rows, :]
            r_scr[:, rows, :] = x
            return x[NT - 1]
        return run

    def block0():
        tm = TM0
        z = z_smem[0]
        for r in range(0, tm, 32):
            if r == tm // 2:
                wait(1)
            if r == tm - 96:
                wait(2)
            store_packed(xn_scr, pl.ds(r // 2, 16), 0, ln_rows(r, 32))
        gu_chunk(tm, 0, True, z=z)
        wait(3)
        gu_chunk(tm, 1, True)
        wait(4)
        gu_chunk(tm, TAIL, True)
        gu_chunk(tm, 2, True)
        prep_qkv(0)
        proj(tm, 0)
        w0[...] = u32(wgu_v[2 * FM:2 * F, :].astype(F32).T.astype(BF16))
        wait(5)
        gu_chunk(tm, 3, True)
        prep_qkv(1)
        proj(tm, 1)
        prep_qkv(2)
        proj(tm, 2)

        def last_region(i, carry):
            wait(6)
            extra = dict(enumerate(prep_table_pieces(z), EXTRA0))
            pace = Pacer(tm, 2, att_tasks(tm, True, z, T00, SPAN0, TP0, 0, extra))
            prep_wo()
            head = passes(2, dot_nn, h_k(tm), lambda k: d_w(True, k, 0), pace)
            for ci in (4, 5, 6):
                gu_chunk(tm, ci, True, pace)
            finish(tm, down(tm, True, pace, head), pace)
            return carry

        lax.fori_loop(0, z + 1, last_region, 0)

    def block(b, carry):
        tm = TM1
        x_wait()
        z = z_smem[0]
        tq, tg, td = 80, 210, 275
        done, back = [], []
        tasks = att_tasks(tm, False, z, tq, SPAN, TPUB, b + 1,
                          {2 * c: residual(TM1 // 16 - 1 - c) for c in range(TM1 // 16)}, done, back)
        npc = FT // PB
        wins = [(TS, tq, G1 * npc), (tq + SPAN + TW2, tg + TG, P2),
                (tg + TG, td + TE, ((XR + TM1) // 16 - G1 - G4) * npc - P2), (td + TE, td + T4, G4 * npc)]
        tasks += tail_tasks(z, b, wins, done, back)
        pace = Pacer(tm, 0, tasks)
        g_scr[XR:XR + tm, :] = passes(NT, dot_nn, xn_k(tm), lambda k: b16(w0[k * 64:(k + 1) * 64, :]), pace)
        for p in range(3):
            proj(tm, p, pace)
        for ci in range(TAIL):
            gu_chunk(tm, ci, False, pace)
        finish(tm, down(tm, False, pace), pace, TM0 + b * TM1, b * XR)
        return carry

    def body(b, carry):
        return block(b, carry)

    def outer(i, carry):
        block0()
        return lax.fori_loop(0, NB1, body, carry)

    for g in groups:
        for c in g:
            c.start()
    xq[2 * TM1 + 16:, 0:128] = jnp.zeros((16, 128), BF16)
    a_scr[NT:3 * NT, 0:HALO, :] = jnp.zeros((2 * NT, HALO, 128), F32)
    wait(0)
    lax.fori_loop(0, z_smem[0] + 1, outer, 0)
    x_wait()
    out_copy(out0_v, pl.ds(0, TM0), pl.ds(0, D)).wait()
    out_copy(out_v, pl.ds(TM0, S - TM0), pl.ds(0, D)).wait()


@jax.jit
def pallas_parallel_sum__sliding_local_dilated__geglu_ffn__prompt_kernel(
        A_x, A_wqkv, A_wo, B_x, B_w_gate, B_w_up, B_w_down):
    hbm = pl.BlockSpec(memory_space=pl.ANY)
    out = pl.pallas_call(
        kernel,
        in_specs=[hbm] * 6,
        out_specs=hbm,
        out_shape=jax.ShapeDtypeStruct((S, D), BF16),
        scratch_shapes=[
            pltpu.VMEM((TM0, D), BF16),
            pltpu.VMEM((2 * TM1 + 32, D), BF16),
            pltpu.VMEM((D, 3 * D), BF16),
            pltpu.VMEM((D, D), BF16),
            pltpu.VMEM((2 * F, D), BF16),
            pltpu.VMEM((F, D), BF16),
            pltpu.VMEM((TM0, D), BF16),
            pltpu.VMEM((S, D), BF16),
            pltpu.VMEM((NT, D // 2, 128), U32),
            pltpu.VMEM((TM0 // 2, D), U32),
            pltpu.VMEM((TM1 // 2 + 8, D), U32),
            pltpu.VMEM((3 * D // 2, D), U32),
            pltpu.VMEM((D // 2, D), U32),
            pltpu.VMEM((FM, D), U32),
            pltpu.VMEM((FM // 2, D), U32),
            pltpu.VMEM((D // 2, 128), U32),
            pltpu.VMEM((TM0 // 2, FM), U32),
            pltpu.VMEM((3, NT, D, 128), F32),
            pltpu.VMEM((4 * NT + 1, TM0 + HALO, 128), F32),
            pltpu.VMEM((FT * NT * 8 + 8, 128), F32),
            pltpu.VMEM((XR + TM1 + 8, 128), F32),
            pltpu.VMEM((NBABY, XR + TM1, 128), F32),
            pltpu.VMEM((NT, XR + TM1, 128), F32),
            pltpu.VMEM((NT, TM0, 128), F32),
            pltpu.VMEM((TM0, 128), F32),
            pltpu.SMEM((1,), jnp.int32),
            pltpu.SemaphoreType.DMA((7,)),
            pltpu.SemaphoreType.DMA((1,)),
            pltpu.SemaphoreType.DMA((1,)),
        ],
        compiler_params=pltpu.CompilerParams(
            vmem_limit_bytes=100 * 1024 * 1024, disable_bounds_checks=True, disable_semaphore_checks=True),
    )(A_x.reshape(S, D), A_wqkv, A_wo, B_w_gate.T, B_w_up.T, B_w_down)
    return out.reshape(1, S, D)
```

```python
import functools
import math
import jax
import jax.numpy as jnp
from jax import lax
import jax.experimental.pallas as pl
import jax.experimental.pallas.tpu as pltpu

S, D, F, H, DH, W, DIL = 2048, 640, 1728, 32, 20, 8, 2
NT = D // 128
TM0 = 512
TM1 = 384
NB1 = (S - TM0) // TM1
XR = TM0 // NB1
HALO = 16
FM = 1664
FT = F - FM
QSCALE = DH ** -0.5 * math.log2(math.e)
NEG = -1e9 * DH ** 0.5
GELU_C1 = math.sqrt(2.0 / math.pi)
GELU_C2 = GELU_C1 * 0.044715
F32, BF16, U32 = jnp.float32, jnp.bfloat16, jnp.uint32
RA = 8
NBABY, NGIANT = 16, 4
PB = 4

SW = 2
T00 = 4
SPAN0 = 120
EXTRA0 = 39
TP0 = 72
PUBT0 = 18
SPAN = 111
TPUB = 216
PUBT = 23
TS = 4
G1 = 15
TW2 = 0
P2 = 48
TG = 1
G4 = 3
TE = 0
T4 = 20
BACKD = 14

CHUNKS = [(0, 128), (128, 256), (384, 128), (512, 384), (896, 256), (1152, 256), (1408, 256), (FM, FT)]
TAIL = len(CHUNKS) - 1


def dot_nn(a, b):
    return jnp.dot(a, b, preferred_element_type=F32)


def dot_nt(a, b):
    return lax.dot_general(a, b, (((1,), (1,)), ((), ())), preferred_element_type=F32)


def geglu2(g, u):
    inner = g * (GELU_C1 + GELU_C2 * (g * g))
    a = g * u
    return a + a * jnp.tanh(inner)


def b16(v):
    return pltpu.bitcast(v, BF16)


def u32(v):
    return pltpu.bitcast(v, U32)


def lanes(j):
    return slice(j * 128, (j + 1) * 128)


def store_packed(ref, rows, col0, v):
    for c in range(0, v.shape[1], 128):
        ref[rows, col0 + c:col0 + c + 128] = u32(v[:, c:c + 128].astype(BF16))


class Pacer:
    def __init__(self, tm, passes, tasks):
        self.tm, self.passes = tm, passes
        self.tasks = sorted(tasks, key=lambda t: t[0])

    def __call__(self, part, k):
        rnd = self.passes // 4
        self.passes += 1
        while k != 1 and self.tasks and self.tasks[0][0] < 4 * (rnd + 1):
            t, fn = self.tasks.pop(0)
            frac = max(0.0, (t - 4 * rnd) / 4)
            tr = min(self.tm - 8, int(frac * self.tm) // 8 * 8)
            fn(part[tr:tr + 8])


def kernel(x_hbm, wqkv_hbm, wo_hbm, wgt_hbm, wut_hbm, wd_hbm, out_hbm,
           x0_v, xq, wqkv_v, wo_v, wgu_v, wd_v, out0_v, out_v,
           u_scr, xn_scr, nx_scr, wqkvp, wop, wgup, wdp, w0, h_scr,
           t_scr, a_scr, v_scr, g_scr, b_scr, r_scr, keep,
           g0_scr, z_smem, sem_i, sem_x, sem_o):
    z_smem[0] = 0

    def out_copy(buf, rows, cols):
        return pltpu.make_async_copy(buf.at[rows, cols], out_hbm.at[rows, cols], sem_o.at[0])

    def x_copy(lo, hi):
        return [(x_hbm.at[pl.ds(lo, hi - lo)], x0_v.at[pl.ds(lo, hi - lo)])]

    def x_block(b, slot):
        row = TM0 + min(b, NB1 - 1) * TM1 if isinstance(b, int) else pl.multiple_of(
            TM0 + jnp.minimum(b, NB1 - 1) * TM1, 16)
        return x_hbm.at[pl.ds(row, TM1)], xq.at[pl.ds(slot * TM1, TM1)]

    def x_refill(b, z):
        for slot in range(2):
            pltpu.make_async_copy(*x_block(b + 1 - slot, slot), sem_x.at[0]).start()
        return xq[pl.ds(pl.multiple_of(2 * TM1 + 16 + z, 16), 16), 0:128].astype(F32)

    def x_wait():
        for slot in range(2):
            pltpu.make_async_copy(*x_block(0, slot), sem_x.at[0]).wait()

    def gu_copy(ci):
        c0, cs = CHUNKS[ci]
        return [(wgt_hbm.at[pl.ds(c0, cs)], wgu_v.at[pl.ds(2 * c0, cs)]),
                (wut_hbm.at[pl.ds(c0, cs)], wgu_v.at[pl.ds(2 * c0 + cs, cs)])]

    def wqkv_copy(lo, hi):
        return [(wqkv_hbm.at[:, pl.ds(lo * D, (hi - lo) * D)], wqkv_v.at[:, pl.ds(lo * D, (hi - lo) * D)])]

    groups = [
        x_copy(0, TM0 // 2),
        x_copy(TM0 // 2, TM0),
        gu_copy(0),
        gu_copy(1),
        gu_copy(2) + gu_copy(TAIL) + wqkv_copy(0, 1),
        gu_copy(3) + wqkv_copy(1, 3),
        gu_copy(4) + gu_copy(5) + gu_copy(6) + [x_block(0, 0), (wo_hbm, wo_v), (wd_hbm, wd_v)],
    ]
    groups = [[pltpu.make_async_copy(src, dst, sem_i.at[g]) for src, dst in grp] for g, grp in enumerate(groups)]

    def wait(g):
        for c in groups[g]:
            c.wait()

    def fence_x(val8, z):
        xq[pl.ds(pl.multiple_of(2 * TM1 + z, 8), 8), 0:128] = val8.astype(BF16)

    def fence_n(val8, z):
        nx_scr[pl.ds(pl.multiple_of(TM1 // 2 + z, 8), 8), 0:128] = u32(val8)

    def fence_a(val8, z):
        a_scr[3 * NT, pl.ds(pl.multiple_of(z, 8), 8), :] = val8

    def fence_v(val8, z):
        v_scr[pl.ds(pl.multiple_of(FT * NT * 8 + z, 8), 8), :] = val8

    def fence_g(val8, z):
        g_scr[pl.ds(pl.multiple_of(XR + TM1 + z, 8), 8), :] = val8

    def rnd(v):
        return v.astype(BF16).astype(F32)

    def wide(v):
        return jnp.concatenate([v] * NT, axis=1)

    def ln_mean(x):
        m = jnp.broadcast_to(jnp.sum(x, axis=-1, keepdims=True) * (1.0 / D), (x.shape[0], 128))
        mb = rnd(m)
        return mb, (m - mb) * (m - mb)

    def ln_rstd(xc, dd):
        var = jnp.broadcast_to(jnp.sum(xc * xc, axis=-1, keepdims=True) * (1.0 / D), dd.shape) - dd
        v = rnd(rnd(jnp.maximum(var, 0.0)) + 1e-5)
        std = rnd(v * lax.rsqrt(v))
        inv = pl.reciprocal(std, approx=True)
        return inv * (2.0 - std * inv)

    def ln_rows(r, n):
        x = x0_v[r:r + n, :].astype(F32)
        mb, dd = ln_mean(x)
        xc = x - wide(mb)
        return rnd(xc) * wide(ln_rstd(xc, dd))

    def ln_x(c):
        return xq[c * 16:(c + 1) * 16, :].astype(F32)

    def ln_apply(c, m, rs):
        y = rnd(ln_x(c) - wide(m)) * wide(rs)
        store_packed(nx_scr, pl.ds(c * 8, 8), 0, y)
        return y[:, 0:128]

    def prep_qkv(p):
        for c in range(NT):
            bt = wqkv_v[:, lanes(p * NT + c)].astype(F32).T
            for j in range(NT):
                t_scr[p, j, lanes(c), :] = bt[:, lanes(j)]
        for d in range(DH):
            for j in range(NT):
                rows = t_scr[p, j, pl.ds(d, H, stride=DH), :]
                wqkvp[(p * D + d * H) // 2:(p * D + (d + 1) * H) // 2, lanes(j)] = u32(rows.astype(BF16))

    def prep_wo():
        for j in range(NT):
            u_scr[j, 0:D // 2, :] = u32(wo_v[:, lanes(j)])
            for e in range(DH // 2):
                a = u_scr[j, pl.ds(e, H // 2, stride=DH), :]
                b = u_scr[j, pl.ds(DH // 2 + e, H // 2, stride=DH), :]
                wop[e * H:e * H + H // 2, lanes(j)] = (a & U32(0xFFFF)) | (b << 16)
                wop[e * H + H // 2:(e + 1) * H, lanes(j)] = (a >> 16) | (b & U32(0xFFFF0000))

    def prep_table_pieces(z):
        def skew(j):
            def run():
                m = 0.5 * wd_v[FM:F, lanes(j)].astype(F32)
                lane = lax.broadcasted_iota(jnp.int32, (FT, 128), 1)
                for bit in range(6):
                    sh = 1 << bit
                    up = jnp.concatenate([m[sh:], m[:sh]], axis=0) if sh % 8 == 0 else pltpu.roll(m, FT - sh, 0)
                    m = jnp.where((lane & sh) != 0, up, m)
                for a in range(NGIANT):
                    blk = m[a * NBABY:(a + 1) * NBABY]
                    t_scr[2, j, a * NBABY:(a + 1) * NBABY, :] = pltpu.roll(blk, a * NBABY, 1) if a else blk
                return jnp.sum(m.reshape(FT // 8, 8, 128), axis=0)
            return run

        def spread(j, a):
            def run():
                blk = t_scr[2, j, a * NBABY:(a + 1) * NBABY, :]
                for b in range(NBABY):
                    r0 = ((a * NBABY + b) * NT + j) * 8
                    v_scr[r0:r0 + 8, :] = jnp.broadcast_to(blk[b:b + 1], (8, 128))
                return v_scr[pl.ds(pl.multiple_of(z, 8), 8), :]
            return run

        return [skew(j) for j in range(NT)] + [spread(j, a) for j in range(NT) for a in range(NGIANT)]

    def gu_w(first, r0, n, cols=slice(None)):
        if not first:
            return b16(wgup[r0 // 2:(r0 + n) // 2, cols])
        w = wgu_v[r0:r0 + n, cols]
        wgup[r0 // 2:(r0 + n) // 2, cols] = u32(w)
        return w

    def d_w(first, k, j):
        if not first:
            return b16(wdp[k * 64:(k + 1) * 64, lanes(j)])
        w = wd_v[lanes(k), lanes(j)]
        wdp[k * 64:(k + 1) * 64, lanes(j)] = u32(w)
        return w

    def passes(n, dot, lhs, rhs, pace, y=None, k0=0):
        for k in range(k0, n):
            part = dot(lhs(k), rhs(k))
            y = part if y is None else y + part
            pace(part, k)
        return y

    def xn_k(tm):
        return lambda k: b16(xn_scr[0:tm // 2, lanes(k)])

    def proj(tm, p, pace=None):
        if pace is None:
            y = dot_nt(b16(xn_scr[0:tm // 2, :]), b16(wqkvp[p * D // 2:(p + 1) * D // 2, :]))
        for j in range(NT):
            r0 = (p * NT + j) * 64
            a_scr[p * NT + j, HALO:HALO + tm, :] = y[:, lanes(j)] if pace is None else passes(
                NT, dot_nt, xn_k(tm), lambda k: b16(wqkvp[r0:r0 + 64, lanes(k)]), pace)

    def gu_chunk(tm, ci, first, pace=None, z=None):
        c0, cs = CHUNKS[ci]
        if pace is not None:
            for t in range(cs // 128):
                g, u = [passes(NT, dot_nt, xn_k(tm), lambda k: gu_w(first, r0, 128, lanes(k)), pace)
                        for r0 in (2 * c0 + t * 128, 2 * c0 + cs + t * 128)]
                store_packed(h_scr, pl.ds(0, tm // 2), c0 + t * 128, geglu2(g, u))
        elif ci == TAIL:
            g0_scr[...] = dot_nt(b16(xn_scr[0:tm // 2, :]), wgu_v[2 * c0:2 * c0 + 2 * cs, :])
        else:
            w = gu_w(first, 2 * c0, 2 * cs)
            if z is None:
                gu = dot_nt(b16(xn_scr[0:tm // 2, :]), w)
            else:
                gu = jnp.concatenate([
                    dot_nt(b16(xn_scr[0:tm // 4, :]), w),
                    dot_nt(b16(xn_scr[tm // 4:tm // 2, :]), wgu_v[pl.ds(pl.multiple_of(2 * c0 + z, 16), 2 * cs), :])],
                    axis=0)
            store_packed(h_scr, pl.ds(0, tm // 2), c0, geglu2(gu[:, :cs], gu[:, cs:]))

    def h_k(tm):
        return lambda k: b16(h_scr[0:tm // 2, lanes(k)])

    def down(tm, first, pace, head=None):
        return [passes(FM // 128, dot_nn, h_k(tm), lambda k: d_w(first, k, j), pace,
                       *((head, 2) if j == 0 and head is not None else ()))
                for j in range(NT)]

    def finish(tm, acc, pace, row0=None, x0=None):
        o = [b16(a_scr[3 * NT + 1 + k, 0:tm // 2, :]) for k in range(NT)]
        for j in range(NT):
            y = passes(NT, dot_nn, lambda k: o[k], lambda k: b16(wop[k * 64:(k + 1) * 64, lanes(j)]), pace)
            if row0 is None:
                keep[j] = 0.5 * acc[j] + x0_v[:, lanes(j)].astype(F32) + y
                continue
            n = tm // 2 if j == NT - 1 else tm
            for r in range(0, tm, n):
                rows = pl.ds(pl.multiple_of(row0 + r, 16), n)
                res = 0.5 * acc[j][r:r + n] + r_scr[j, XR + r:XR + r + n, :]
                out_v[rows, lanes(j)] = (res + y[r:r + n]).astype(BF16)
                if j == NT - 1 and r + n == tm:
                    out_copy(out0_v, pl.ds(pl.multiple_of(x0 + XR - 16 * G4, 16), 16 * G4), pl.ds(0, D)).start()
                out_copy(out_v, rows, pl.ds(j * 128, 128)).start()
        assert not pace.tasks

    def att_qk(first, r, z):
        q = a_scr[0:NT, HALO + r:HALO + r + RA, :]
        s = []
        for w in range(W):
            lo = HALO + r - DIL * w
            sw = jnp.sum(q * a_scr[NT:2 * NT, lo:lo + RA, :], axis=0)
            if (w + 1) % SW == 0:
                fence_a(sw, z)
            t = sw + pltpu.roll(sw, 64, 1)
            s.append(t + pltpu.roll(t, 32, 1))
        if first and r < DIL * (W - 1):
            pos = r + lax.broadcasted_iota(jnp.int32, (RA, 128), 0)
            s = [jnp.where(pos >= DIL * w, s[w], NEG) for w in range(W)]
        return s

    def att_pv(r, z, s):
        mx = functools.reduce(jnp.maximum, s)
        p = [jnp.exp2((l - mx) * QSCALE) for l in s]
        den = functools.reduce(lambda a, b: a + b, p)
        inv = pl.reciprocal(den, approx=True)
        inv = inv * (2.0 - den * inv)
        o = None
        for w in range(W):
            lo = HALO + r - DIL * w
            t = p[w][None] * a_scr[2 * NT:3 * NT, lo:lo + RA, :]
            o = t if o is None else o + t
            if (w + 1) % SW == 0 and w < W - 1:
                fence_a(o[NT - 1], z)
        o = o * inv[None]
        if r % 16 == 0:
            a_scr[0:NT, pl.ds(pl.multiple_of(HALO + r + z, 8), RA), :] = o
        else:
            both = jnp.concatenate([a_scr[0:NT, HALO + r - RA:HALO + r, :], o], axis=1)
            for j in range(NT):
                a_scr[3 * NT + 1 + j, pl.ds(pl.multiple_of((r - RA) // 2 + z, 8), 8), :] = pltpu.bitcast(
                    both[j].astype(BF16), F32)
        return o[0]

    def att_tasks(tm, first, z, t0, span, tpub, nb, extra, done=None, back=None):
        na = tm // RA
        nln = TM1 // 16
        n = max(na + 1, 2 * nln + 2)
        links, pend, m, dd, rs = [], [], {}, {}, {}

        def step(i):
            def run(trig):
                c = i // 2
                fence_a(trig, z)
                if c <= nln:
                    fence_x(trig, z)
                for _, v in [l for l in links if l[0] <= i]:
                    for r in range(0, v.shape[0], 8):
                        fence_a(v[r:r + 8], z)
                links[:] = [l for l in links if l[0] > i]
                if done:
                    links.append((i + 1, done[-1]))
                    done.clear()
                if i % 2 == 0:
                    if c < nln:
                        m[c], dd[c] = ln_mean(ln_x(c))
                        links.append((i + 1, m[c]))
                else:
                    if 0 < c <= nln:
                        links.append((i + 1, ln_apply(c - 1, m[c - 1], rs[c - 1])))
                    if c == nln:
                        links.append((i + 1, x_refill(nb, z)))
                    if c < nln:
                        rs[c] = ln_rstd(ln_x(c) - wide(m[c]), dd[c])
                        links.append((i + 2, rs[c]))
                if i in extra:
                    links.append((i + 2, extra.pop(i)()))
                if i < na:
                    pend.append(att_qk(first, i * RA, z))
                if 1 <= i <= na:
                    last = att_pv((i - 1) * RA, z, pend.pop(0))
                    if back is not None:
                        back[:] = [last]
                if i == n - 1:
                    assert not extra
                    for _, v in links:
                        if back is not None:
                            back[0] = back[0] + v[0:8] + v[v.shape[0] - 8:]
                    a_scr[NT:3 * NT, 0:HALO, :] = a_scr[NT:3 * NT, tm:tm + HALO, :]
            return run

        def publish(c):
            def run(trig):
                fence_n(trig, z)
                xn_scr[c * 8:(c + 1) * 8, :] = nx_scr[c * 8:(c + 1) * 8, :]
            return run

        tasks = [(t0 + span * i / n, step(i)) for i in range(n)]
        t = tpub
        for c in range(nln):
            t = max(t, t0 + span * (2 * c + 4.5) / n)
            tasks.append((t, publish(c)))
            t += (PUBT0 if first else PUBT) / 10
        return tasks

    def tail_tasks(z, b, wins, done, back):
        x0 = pl.multiple_of(b * XR, 16)
        g_scr[0:XR, :] = g0_scr[pl.ds(x0, XR), :]
        r_scr[:, 0:XR, :] = keep[:, pl.ds(x0, XR), :]
        times = []
        for lo, hi, num in wins:
            times += [lo + (hi - lo) * i / num for i in range(num)]
        npc = FT // PB
        assert len(times) == (XR + TM1) // 16 * npc
        st = dict(acc=None, tot=None, n=0)
        links = []

        def rolls(g):
            def run(trig):
                if trig is not None:
                    fence_g(trig, z)
                gu = g_scr[g * 16:(g + 1) * 16, :]
                ru = pltpu.roll(gu, FT, 1)
                low = lax.broadcasted_iota(jnp.int32, gu.shape, 1) < FT
                hh = geglu2(jnp.where(low, gu, ru), jnp.where(low, ru, gu))
                b_scr[0, g * 16:(g + 1) * 16, :] = hh
                for i in range(1, NBABY):
                    b_scr[i, g * 16:(g + 1) * 16, :] = pltpu.roll(hh, 128 - i, 1)
            return run

        def piece(g, s0):
            def run(trig):
                st["n"] += 1
                if back and s0 == 0:
                    links.append((st["n"] + BACKD, back.pop()))
                for _, v in [l for l in links if l[0] <= st["n"]]:
                    trig = trig + v
                links[:] = [l for l in links if l[0] > st["n"]]
                fence_v(trig, z)
                for s in range(s0, s0 + PB):
                    a, i = divmod(s, NBABY)
                    rb = b_scr[i, g * 16:(g + 1) * 16, :].reshape(1, 2, 8, 128)
                    t = rb * v_scr[s * NT * 8:(s + 1) * NT * 8, :].reshape(NT, 1, 8, 128)
                    st["acc"] = t if i == 0 else st["acc"] + t
                    if i == NBABY - 1:
                        acc = st["acc"].reshape(NT * 16, 128)
                        st["tot"] = acc if a == 0 else st["tot"] + pltpu.roll(acc, 128 - a * NBABY, 1)
                v = jnp.sum(st["acc"].reshape(2 * NT, 8, 128), axis=0)
                links.append((st["n"] + 2, v))
                done.append(v)
                if s0 + PB == FT:
                    tot = st["tot"].reshape(NT, 16, 128)
                    if g < XR // 16:
                        rows = pl.ds(pl.multiple_of(x0 + g * 16, 16), 16)
                        tot = tot + r_scr[:, g * 16:(g + 1) * 16, :]
                        out0_v[rows, :] = jnp.concatenate([tot[j] for j in range(NT)], axis=1).astype(BF16)
                        if g == XR // 16 - G4 - 1:
                            out_copy(out0_v, pl.ds(pl.multiple_of(x0, 16), XR - 16 * G4), pl.ds(0, D)).start()
                    else:
                        if st["n"] > G1 * npc:
                            tot = tot + r_scr[:, g * 16:(g + 1) * 16, :]
                        r_scr[:, g * 16:(g + 1) * 16, :] = tot
                    links.append((st["n"] + 8, jnp.sum(tot.reshape(2 * NT, 8, 128), axis=0)))
            return run

        nx = XR // 16
        order = list(range(nx - G4)) + list(range(nx, nx + TM1 // 16)) + list(range(nx - G4, nx))
        rolls(order[0])(None)
        tasks = []
        for q, g in enumerate(order):
            if q:
                tasks.append((times[(q - 1) * npc] + 0.01, rolls(g)))
            for i in range(npc):
                tasks.append((times[q * npc + i], piece(g, i * PB)))
        return tasks

    def residual(c):
        def run():
            x = xq[TM1 + c * 16:TM1 + (c + 1) * 16, :].astype(F32)
            x = jnp.stack([x[:, lanes(j)] for j in range(NT)])
            rows = slice(XR + c * 16, XR + (c + 1) * 16)
            if c < G1 - (XR // 16 - G4):
                x = x + r_scr[:, rows, :]
            r_scr[:, rows, :] = x
            return x[NT - 1]
        return run

    def block0():
        tm = TM0
        z = z_smem[0]
        for r in range(0, tm, 32):
            if r == tm // 2:
                wait(1)
            if r == tm - 96:
                wait(2)
            store_packed(xn_scr, pl.ds(r // 2, 16), 0, ln_rows(r, 32))
        gu_chunk(tm, 0, True, z=z)
        wait(3)
        gu_chunk(tm, 1, True)
        wait(4)
        gu_chunk(tm, TAIL, True)
        gu_chunk(tm, 2, True)
        prep_qkv(0)
        proj(tm, 0)
        w0[...] = u32(wgu_v[2 * FM:2 * F, :].astype(F32).T.astype(BF16))
        wait(5)
        gu_chunk(tm, 3, True)
        prep_qkv(1)
        proj(tm, 1)
        prep_qkv(2)
        proj(tm, 2)

        def last_region(i, carry):
            wait(6)
            extra = dict(enumerate(prep_table_pieces(z), EXTRA0))
            pace = Pacer(tm, 2, att_tasks(tm, True, z, T00, SPAN0, TP0, 0, extra))
            prep_wo()
            head = passes(2, dot_nn, h_k(tm), lambda k: d_w(True, k, 0), pace)
            for ci in (4, 5, 6):
                gu_chunk(tm, ci, True, pace)
            finish(tm, down(tm, True, pace, head), pace)
            return carry

        lax.fori_loop(0, z + 1, last_region, 0)

    def block(b, carry):
        tm = TM1
        x_wait()
        z = z_smem[0]
        tq, tg, td = 80, 210, 275
        done, back = [], []
        tasks = att_tasks(tm, False, z, tq, SPAN, TPUB, b + 1,
                          {2 * c: residual(TM1 // 16 - 1 - c) for c in range(TM1 // 16)}, done, back)
        npc = FT // PB
        wins = [(TS, tq, G1 * npc), (tq + SPAN + TW2, tg + TG, P2),
                (tg + TG, td + TE, ((XR + TM1) // 16 - G1 - G4) * npc - P2), (td + TE, td + T4, G4 * npc)]
        tasks += tail_tasks(z, b, wins, done, back)
        pace = Pacer(tm, 0, tasks)
        g_scr[XR:XR + tm, :] = passes(NT, dot_nn, xn_k(tm), lambda k: b16(w0[k * 64:(k + 1) * 64, :]), pace)
        for p in range(3):
            proj(tm, p, pace)
        for ci in range(TAIL):
            gu_chunk(tm, ci, False, pace)
        finish(tm, down(tm, False, pace), pace, TM0 + b * TM1, b * XR)
        return carry

    def outer(i, carry):
        block0()
        return lax.fori_loop(0, NB1, block, carry)

    for g in groups:
        for c in g:
            c.start()
    xq[2 * TM1 + 16:, 0:128] = jnp.zeros((16, 128), BF16)
    a_scr[NT:3 * NT, 0:HALO, :] = jnp.zeros((2 * NT, HALO, 128), F32)
    wait(0)
    lax.fori_loop(0, z_smem[0] + 1, outer, 0)
    x_wait()
    out_copy(out0_v, pl.ds(0, TM0), pl.ds(0, D)).wait()
    out_copy(out_v, pl.ds(TM0, S - TM0), pl.ds(0, D)).wait()


@jax.jit
def pallas_parallel_sum__sliding_local_dilated__geglu_ffn__prompt_kernel(
        A_x, A_wqkv, A_wo, B_x, B_w_gate, B_w_up, B_w_down):
    hbm = pl.BlockSpec(memory_space=pl.ANY)
    out = pl.pallas_call(
        kernel,
        in_specs=[hbm] * 6,
        out_specs=hbm,
        out_shape=jax.ShapeDtypeStruct((S, D), BF16),
        scratch_shapes=[
            pltpu.VMEM((TM0, D), BF16),
            pltpu.VMEM((2 * TM1 + 32, D), BF16),
            pltpu.VMEM((D, 3 * D), BF16),
            pltpu.VMEM((D, D), BF16),
            pltpu.VMEM((2 * F, D), BF16),
            pltpu.VMEM((F, D), BF16),
            pltpu.VMEM((TM0, D), BF16),
            pltpu.VMEM((S, D), BF16),
            pltpu.VMEM((NT, D // 2 + 24, 128), U32),
            pltpu.VMEM((TM0 // 2, D), U32),
            pltpu.VMEM((TM1 // 2 + 8, D), U32),
            pltpu.VMEM((3 * D // 2, D), U32),
            pltpu.VMEM((D // 2, D), U32),
            pltpu.VMEM((FM, D), U32),
            pltpu.VMEM((FM // 2, D), U32),
            pltpu.VMEM((D // 2, 128), U32),
            pltpu.VMEM((TM0 // 2, FM), U32),
            pltpu.VMEM((3, NT, D + 32, 128), F32),
            pltpu.VMEM((4 * NT + 1, TM0 + HALO + 24, 128), F32),
            pltpu.VMEM((FT * NT * 8 + 8, 128), F32),
            pltpu.VMEM((XR + TM1 + 8, 128), F32),
            pltpu.VMEM((NBABY, XR + TM1, 128), F32),
            pltpu.VMEM((NT, XR + TM1, 128), F32),
            pltpu.VMEM((NT, TM0, 128), F32),
            pltpu.VMEM((TM0, 128), F32),
            pltpu.SMEM((1,), jnp.int32),
            pltpu.SemaphoreType.DMA((7,)),
            pltpu.SemaphoreType.DMA((1,)),
            pltpu.SemaphoreType.DMA((1,)),
        ],
        compiler_params=pltpu.CompilerParams(
            vmem_limit_bytes=100 * 1024 * 1024, disable_bounds_checks=True, disable_semaphore_checks=True),
    )(A_x.reshape(S, D), A_wqkv, A_wo, B_w_gate.T, B_w_up.T, B_w_down)
    return out.reshape(1, S, D)
```
